```python
import jax
import jax.numpy as jnp

def _softmax(x, axis=-1):
    return jax.nn.softmax(x, axis=axis)

def _gelu(x):
    return jax.nn.gelu(x, approximate=True)

def _silu(x):
    return jax.nn.silu(x)

def _sigmoid(x):
    return jax.nn.sigmoid(x)

def _layernorm(x, axis=-1, eps=1e-05):
    m = jnp.mean(x, axis=axis, keepdims=True)
    v = jnp.var(x, axis=axis, keepdims=True)
    return (x - m) / jnp.sqrt(v + eps)

def _scatter_add(tgt, idx, src, axis=0):
    return tgt.at[idx].add(src)

def _segment_sum(src, seg, n):
    return jax.ops.segment_sum(src, seg, n)

class _Rng:

    def __init__(self, key):
        self._k = key

    def _next(self):
        self._k, sub = jax.random.split(self._k)
        return sub

    def normal(self, shape):
        return jax.random.normal(self._next(), shape, dtype=jnp.bfloat16)

    def randint(self, lo, hi, shape):
        return jax.random.randint(self._next(), shape, lo, hi, dtype=jnp.int32)

    def uniform(self, shape, lo=0.0, hi=1.0):
        return jax.random.uniform(self._next(), shape, jnp.bfloat16, lo, hi)

    def permutation(self, n):
        return jax.random.permutation(self._next(), n)
kernel_name = 'interleave_layers__memory_aug_recurrent_mem_tr__glu_gated_swiglu__prompt'

def setup_inputs():
    _rng = _Rng(jax.random.key(int.from_bytes(__import__("os").urandom(4), "little")))
    _w = lambda a: (lambda t: t.astype(jnp.bfloat16) if jnp.issubdtype(t.dtype, jnp.floating) else t)(jnp.asarray(a))

    def _A_setup():
        B, S, Dm = (1, 2048, 576)
        H, Dh = (32, 128)
        M, seg = (8, 32)
        seg = min(seg, S)
        S = S // seg * seg
        return {'x': _w((lambda *s: _rng.normal(s) * 0.05)(B, S, Dm)), 'mem0': _w((lambda *s: _rng.normal(s) * 0.05)(B, M, Dm)), 'Wq': _w((lambda *s: _rng.normal(s) * 0.05)(Dm, H, Dh) * Dm ** (-0.5)), 'Wk': _w((lambda *s: _rng.normal(s) * 0.05)(Dm, H, Dh) * Dm ** (-0.5)), 'Wv': _w((lambda *s: _rng.normal(s) * 0.05)(Dm, H, Dh) * Dm ** (-0.5)), 'Wo': _w((lambda *s: _rng.normal(s) * 0.05)(H, Dh, Dm) * (H * Dh) ** (-0.5)), 'seg_len': seg}
    _A_in = _A_setup()

    def _B_setup():
        B, S, D, F = (1, 2048, 576, 4608)
        return {'x': _w((lambda *s: _rng.normal(s) * 0.05)(B, S, D)), 'w1': _w((lambda *s: _rng.normal(s) * 0.05)(D, F) * (2.0 / D) ** 0.5), 'w3': _w((lambda *s: _rng.normal(s) * 0.05)(D, F) * (2.0 / D) ** 0.5), 'w2': _w((lambda *s: _rng.normal(s) * 0.05)(F, D) * (2.0 / F) ** 0.5)}
    _B_in = _B_setup()
    return {'A_x': _A_in['x'], 'A_mem0': _A_in['mem0'], 'A_Wq': _A_in['Wq'], 'A_Wk': _A_in['Wk'], 'A_Wv': _A_in['Wv'], 'A_Wo': _A_in['Wo'], 'A_seg_len': _A_in['seg_len'], 'B_x': _B_in['x'], 'B_w1': _B_in['w1'], 'B_w3': _B_in['w3'], 'B_w2': _B_in['w2']}

def reference(A_x, A_mem0, A_Wq, A_Wk, A_Wv, A_Wo, A_seg_len, B_x, B_w1, B_w3, B_w2):

    def _A_ref(x, mem0, Wq, Wk, Wv, Wo, seg_len):
        B, S, Dm = x.shape
        H, Dh = (Wq.shape[1], Wq.shape[2])
        M = mem0.shape[1]
        scale = Dh ** (-0.5)
        n_seg = S // seg_len
        L = M + seg_len
        idx = jnp.arange(L)
        mask = (idx[:, None] < M) | (idx[:, None] >= idx[None, :])
        mem = mem0
        outs = []
        for s in range(n_seg):
            xs = x[:, s * seg_len:(s + 1) * seg_len, :].copy()
            h = jnp.concatenate([mem, xs], axis=1)
            q = jnp.einsum('btd,dhe->bhte', h, Wq)
            k = jnp.einsum('btd,dhe->bhte', h, Wk)
            v = jnp.einsum('btd,dhe->bhte', h, Wv)
            scores = jnp.einsum('bhqe,bhke->bhqk', q, k) * scale
            scores = jnp.where(mask[None, None], scores, -1000000000.0)
            p = _softmax(scores, axis=-1)
            o = jnp.einsum('bhqk,bhke->bhqe', p, v)
            o = jnp.einsum('bhte,hed->btd', o, Wo)
            mem = o[:, :M, :].copy()
            outs.append(o[:, M:, :])
        return jnp.concatenate(outs, axis=1)

    def _B_ref(x, w1, w3, w2):
        gate = jnp.einsum('bsd,df->bsf', x, w1)
        up = jnp.einsum('bsd,df->bsf', x, w3)
        h = _silu(gate) * up
        out = jnp.einsum('bsf,fd->bsd', h, w2)
        return out
    x = A_x
    x = x + _A_ref(_layernorm(x, axis=-1), A_mem0, A_Wq, A_Wk, A_Wv, A_Wo, A_seg_len)
    x = x + _B_ref(_layernorm(x, axis=-1), B_w1, B_w3, B_w2)
    x = x + _A_ref(_layernorm(x, axis=-1), A_mem0, A_Wq, A_Wk, A_Wv, A_Wo, A_seg_len)
    x = x + _B_ref(_layernorm(x, axis=-1), B_w1, B_w3, B_w2)
    return x
```

```python
import functools
import math

import jax
import jax.numpy as jnp
from jax import lax
import jax.experimental.pallas as pl
import jax.experimental.pallas.tpu as pltpu

F32 = jnp.float32
BF16 = jnp.bfloat16
LANES = 128
LAG = 6
HEAD_GROUP = 2
FF_CHUNK = 512
LN_EPS = 1e-5
MASK_FILL = -1000000000.0
LOG2E = math.log2(math.e)
NT_DIMS = (((1,), (1,)), ((), ()))


def _dot(a, b):
    return jnp.dot(a, b, preferred_element_type=F32)


def _dot_nt(a, b):
    return lax.dot_general(a, b, NT_DIMS, preferred_element_type=F32)


def _layernorm(x):
    mean = jnp.mean(x, axis=-1, keepdims=True)
    cen = x - mean
    var = jnp.mean(cen * cen, axis=-1, keepdims=True)
    return cen * lax.rsqrt(var + LN_EPS)


def _mask_fill(n_streams, seg, n_mem):
    rows = n_streams * (seg + n_mem)

    def stream_and_pos(i):
        is_mem = i >= n_streams * seg
        j = i - n_streams * seg
        stream = jnp.where(is_mem, j // n_mem, i // seg)
        pos = jnp.where(is_mem, j % n_mem, n_mem + i % seg)
        return stream, pos

    q_stream, q_pos = stream_and_pos(lax.broadcasted_iota(jnp.int32, (rows, rows), 0))
    k_stream, k_pos = stream_and_pos(lax.broadcasted_iota(jnp.int32, (rows, rows), 1))
    visible = (q_pos < n_mem) | (q_pos >= k_pos)
    fill = jnp.where(visible, 0.0, MASK_FILL * LOG2E).astype(F32)
    return jnp.where(q_stream == k_stream, fill, -jnp.inf)


def _kernel(xt_hbm, mem0_ref, wq_hbm, wk_hbm, wv_hbm, wot_hbm, w1_hbm, w3_hbm, w2t_hbm,
            out_hbm,
            xt_buf, stage, wqkv, wot, w1, w3, w2t, res, nrm, mem, o_buf, h_buf, ff_acc,
            fill1, fill2, sem_x, sem_qkv, sem_o, sem_ff, sem_out,
            *, seg, n_mem, n_heads, head_dim):
    d_model, seq = xt_buf.shape
    d_ff = w1.shape[1]
    n_seg = seq // seg
    n_pairs = n_heads // 2
    n_groups = n_heads // HEAD_GROUP
    n_chunks = d_ff // FF_CHUNK
    score_scale = head_dim ** -0.5 * LOG2E
    head_cols = 3 * head_dim

    x_copy = pltpu.make_async_copy(xt_hbm, xt_buf, sem_x)

    def qkv_copy(pair, which):
        src = (wq_hbm, wk_hbm, wv_hbm)[which].bitcast(jnp.uint32)
        return pltpu.make_async_copy(src.at[:, pair, :], stage.at[which, pair],
                                     sem_qkv.at[which, pair])

    def wo_copy(head):
        return pltpu.make_async_copy(
            wot_hbm.at[head], wot.at[:, pl.ds(head * head_dim, head_dim)], sem_o.at[head])

    ff_copies = [pltpu.make_async_copy(src, dst, sem_ff.at[i])
                 for i, (src, dst) in enumerate(((w1_hbm, w1), (w3_hbm, w3), (w2t_hbm, w2t)))]

    x_copy.start()
    for pair in range(n_pairs):
        for which in range(3):
            qkv_copy(pair, which).start()
    for head in range(n_heads):
        wo_copy(head).start()
    for copy in ff_copies:
        copy.start()

    fill1[...] = _mask_fill(1, seg, n_mem)
    fill2[...] = _mask_fill(2, seg, n_mem)
    mem0 = mem0_ref[...].astype(F32)
    mem[0:n_mem, :] = mem0
    mem[n_mem:2 * n_mem, :] = mem0

    x_copy.wait()

    def load_tokens(j, carry):
        tok = pl.ds(pl.multiple_of(j * LANES, LANES), LANES)
        x = xt_buf[:, tok].astype(F32).T
        res[tok, :] = x
        nrm[tok, :] = _layernorm(x).astype(BF16)
        return carry

    lax.fori_loop(0, seq // LANES, load_tokens, 0)

    def unpack_pair(pair, carry):
        for which in range(3):
            qkv_copy(pair, which).wait()
            words = stage[which, pair]
            even = lax.bitcast_convert_type(words << 16, F32)
            odd = lax.bitcast_convert_type(words & jnp.uint32(0xFFFF0000), F32)
            for parity, w in enumerate((even, odd)):
                col = (2 * pair + parity) * head_cols + which * head_dim
                wqkv[:, pl.ds(pl.multiple_of(col, LANES), head_dim)] = w.astype(BF16)
        return carry

    lax.fori_loop(0, n_pairs, unpack_pair, 0)
    for head in range(n_heads):
        wo_copy(head).wait()

    def seg_rows(s):
        return pl.ds(pl.multiple_of(s * seg, seg), seg)

    def add_and_normalize(s, delta):
        x = res[seg_rows(s), :] + delta
        res[seg_rows(s), :] = x
        nrm[seg_rows(s), :] = _layernorm(x).astype(BF16)

    def attention_stages(h, fill_ref):
        rows = h.shape[0]
        qkv, probs = {}, {}
        for g in range(n_groups + 2):
            if g < n_groups:
                cols = slice(g * HEAD_GROUP * head_cols, (g + 1) * HEAD_GROUP * head_cols)
                qkv[g] = _dot(h, wqkv[:, cols]).astype(BF16)
            if 0 <= g - 1 < n_groups:
                y = qkv[g - 1]
                probs[g - 1] = []
                for i in range(HEAD_GROUP):
                    q = y[:, i * head_cols:i * head_cols + head_dim]
                    k = y[:, i * head_cols + head_dim:i * head_cols + 2 * head_dim]
                    fill = fill_ref[...]
                    s = jnp.where(fill == 0.0, _dot_nt(q, k) * score_scale, fill)
                    e = jnp.exp2(s - jnp.max(s, axis=-1, keepdims=True))
                    p = e * (1.0 / jnp.sum(e, axis=-1, keepdims=True))
                    probs[g - 1].append(p.astype(BF16))
            if 0 <= g - 2 < n_groups:
                y = qkv.pop(g - 2)
                for i, p in enumerate(probs.pop(g - 2)):
                    v = y[:, i * head_cols + 2 * head_dim:(i + 1) * head_cols]
                    head = (g - 2) * HEAD_GROUP + i
                    o_buf[0:rows, head * head_dim:(head + 1) * head_dim] = _dot(p, v).astype(BF16)
            yield

    def attention_output(rows):
        return _dot_nt(o_buf[0:rows, :], wot[...])

    def gate_up(hf, c):
        cols = slice(c * FF_CHUNK, (c + 1) * FF_CHUNK)
        gate = _dot(hf, w1[:, cols])
        up = _dot(hf, w3[:, cols])
        h_buf[:, cols] = (gate * (1.0 / (1.0 + jnp.exp(-gate))) * up).astype(BF16)

    def ff_input(sa, sb):
        return jnp.concatenate([nrm[seg_rows(sa), :], nrm[seg_rows(sb), :]], axis=0)

    def ff_down():
        ff_acc[...] = _dot_nt(h_buf[...], w2t[...])

    def ff_finish(sa, sb):
        add_and_normalize(sa, ff_acc[0:seg, :])
        add_and_normalize(sb, ff_acc[seg:2 * seg, :])

    def ff_blocks(t):
        head = t <= LAG
        tail = t > n_seg
        sa = jnp.where(head, 2 * (t - LAG // 2 - 1), jnp.where(tail, t - LAG - 2, t - 1))
        sb = jnp.where(head | tail, sa + 1, t - LAG - 1)
        return sa, sb

    first_ff = LAG // 2 + 1
    last_step = n_seg + LAG + 1

    def has_ff(t):
        in_tail = (t > n_seg) & (t < last_step) & ((t - n_seg) % 2 == 0)
        return ((t >= first_ff) & (t <= n_seg)) | in_tail

    def step(t, carry):
        fused = (t >= LAG) & (t < n_seg)

        @pl.when(t == first_ff)
        def _():
            for copy in ff_copies:
                copy.wait()

        @pl.when(fused)
        def _():
            ff_finish(*ff_blocks(t - 1))
            s1, s2 = t, t - LAG
            h = jnp.concatenate(
                [nrm[seg_rows(s1), :], nrm[seg_rows(s2), :], mem[...].astype(BF16)], axis=0)
            hf = ff_input(*ff_blocks(t))
            chunk = 0
            for g, _ in enumerate(attention_stages(h, fill2)):
                if g >= n_groups - 1:
                    gate_up(hf, chunk)
                    chunk += 1
            for c in range(chunk, n_chunks):
                gate_up(hf, c)
            out = attention_output(2 * (seg + n_mem))
            ff_down()
            mem[...] = out[2 * seg:, :]
            add_and_normalize(s1, out[0:seg, :])
            add_and_normalize(s2, out[seg:2 * seg, :])

        @pl.when(jnp.logical_not(fused))
        def _():
            @pl.when(has_ff(t - 1))
            def _():
                ff_finish(*ff_blocks(t - 1))

            @pl.when(t < n_seg + LAG)
            def _():
                second = t >= n_seg
                s = jnp.where(second, t - LAG, t)
                mem_rows = pl.ds(pl.multiple_of(jnp.where(second, n_mem, 0), n_mem), n_mem)
                h = jnp.concatenate(
                    [nrm[seg_rows(s), :].astype(F32), mem[mem_rows, :]], axis=0).astype(BF16)
                for _ in attention_stages(h, fill1):
                    pass
                out = attention_output(seg + n_mem)
                mem[mem_rows, :] = out[seg:, :]
                add_and_normalize(s, out[0:seg, :])

            @pl.when(has_ff(t))
            def _():
                hf = ff_input(*ff_blocks(t))
                for c in range(n_chunks):
                    gate_up(hf, c)
                ff_down()

        return carry

    lax.fori_loop(0, last_step + 1, step, 0)

    def out_copy(j):
        tok = pl.ds(pl.multiple_of(j * LANES, LANES), LANES)
        return pltpu.make_async_copy(xt_buf.at[:, tok], out_hbm.at[:, tok], sem_out.at[j])

    def store_tokens(j, carry):
        tok = pl.ds(pl.multiple_of(j * LANES, LANES), LANES)
        xt_buf[:, tok] = res[tok, :].T.astype(BF16)
        out_copy(j).start()
        return carry

    lax.fori_loop(0, seq // LANES, store_tokens, 0)

    def wait_tokens(j, carry):
        out_copy(j).wait()
        return carry

    lax.fori_loop(0, seq // LANES, wait_tokens, 0)


@functools.partial(jax.jit, static_argnames=("A_seg_len",))
def pallas_interleave_layers__memory_aug_recurrent_mem_tr__glu_gated_swiglu__prompt_kernel(
    A_x: jax.Array,
    A_mem0: jax.Array,
    A_Wq: jax.Array,
    A_Wk: jax.Array,
    A_Wv: jax.Array,
    A_Wo: jax.Array,
    A_seg_len: int,
    B_x: jax.Array,
    B_w1: jax.Array,
    B_w3: jax.Array,
    B_w2: jax.Array,
):
    del B_x
    batch, seq, d_model = A_x.shape
    n_mem = A_mem0.shape[1]
    _, n_heads, head_dim = A_Wq.shape
    d_ff = B_w1.shape[1]
    seg = int(A_seg_len)
    assert batch == 1 and seq % LANES == 0 and seq % seg == 0 and head_dim == LANES
    assert d_ff % FF_CHUNK == 0 and n_heads % HEAD_GROUP == 0 and LAG % 2 == 0
    rows = 2 * (seg + n_mem)

    any_spec = pl.BlockSpec(memory_space=pl.ANY)
    out_t = pl.pallas_call(
        functools.partial(_kernel, seg=seg, n_mem=n_mem, n_heads=n_heads, head_dim=head_dim),
        out_shape=jax.ShapeDtypeStruct((d_model, seq), A_x.dtype),
        in_specs=[any_spec, pl.BlockSpec(memory_space=pltpu.VMEM)] + [any_spec] * 7,
        out_specs=any_spec,
        scratch_shapes=[
            pltpu.VMEM((d_model, seq), BF16),
            pltpu.VMEM((3, n_heads // 2, d_model, head_dim), jnp.uint32),
            pltpu.VMEM((d_model, 3 * n_heads * head_dim), BF16),
            pltpu.VMEM((d_model, n_heads * head_dim), BF16),
            pltpu.VMEM((d_model, d_ff), BF16),
            pltpu.VMEM((d_model, d_ff), BF16),
            pltpu.VMEM((d_model, d_ff), BF16),
            pltpu.VMEM((seq, d_model), F32),
            pltpu.VMEM((seq, d_model), BF16),
            pltpu.VMEM((2 * n_mem, d_model), F32),
            pltpu.VMEM((rows, n_heads * head_dim), BF16),
            pltpu.VMEM((2 * seg, d_ff), BF16),
            pltpu.VMEM((2 * seg, d_model), F32),
            pltpu.VMEM((rows // 2, rows // 2), F32),
            pltpu.VMEM((rows, rows), F32),
            pltpu.SemaphoreType.DMA(()),
            pltpu.SemaphoreType.DMA((3, n_heads // 2)),
            pltpu.SemaphoreType.DMA((n_heads,)),
            pltpu.SemaphoreType.DMA((3,)),
            pltpu.SemaphoreType.DMA((seq // LANES,)),
        ],
        compiler_params=pltpu.CompilerParams(vmem_limit_bytes=100 * 1024 * 1024),
    )(
        A_x[0].T,
        A_mem0[0],
        A_Wq,
        A_Wk,
        A_Wv,
        jnp.transpose(A_Wo, (0, 2, 1)),
        B_w1,
        B_w3,
        B_w2.T,
    )
    return out_t.T[None]
```

```python
import functools
import math

import jax
import jax.numpy as jnp
from jax import lax
import jax.experimental.pallas as pl
import jax.experimental.pallas.tpu as pltpu

F32 = jnp.float32
BF16 = jnp.bfloat16
LANES = 128
LAG = 6
HEAD_GROUP = 2
FF_CHUNK = 512
COPY_WINDOW = 2
LN_EPS = 1e-5
MASK_FILL = -1000000000.0
LOG2E = math.log2(math.e)
NT_DIMS = (((1,), (1,)), ((), ()))


def _dot(a, b):
    return jnp.dot(a, b, preferred_element_type=F32)


def _dot_nt(a, b):
    return lax.dot_general(a, b, NT_DIMS, preferred_element_type=F32)


def _as_bf16(words):
    return pltpu.bitcast(words, BF16)


def _layernorm(x):
    mean = jnp.mean(x, axis=-1, keepdims=True)
    cen = x - mean
    var = jnp.mean(cen * cen, axis=-1, keepdims=True)
    return cen * lax.rsqrt(var + LN_EPS)


def _mask_fill(n_streams, seg, n_mem):
    rows = n_streams * (seg + n_mem)

    def stream_and_pos(i):
        is_mem = i >= n_streams * seg
        j = i - n_streams * seg
        stream = jnp.where(is_mem, j // n_mem, i // seg)
        pos = jnp.where(is_mem, j % n_mem, n_mem + i % seg)
        return stream, pos

    q_stream, q_pos = stream_and_pos(lax.broadcasted_iota(jnp.int32, (rows, rows), 0))
    k_stream, k_pos = stream_and_pos(lax.broadcasted_iota(jnp.int32, (rows, rows), 1))
    visible = (q_pos < n_mem) | (q_pos >= k_pos)
    fill = jnp.where(visible, 0.0, MASK_FILL * LOG2E).astype(F32)
    return jnp.where(q_stream == k_stream, fill, -jnp.inf)


def _kernel(xt_hbm, mem0_ref, wq_hbm, wk_hbm, wv_hbm, wot_hbm, w1_hbm, w3_hbm, w2t_hbm,
            out_hbm,
            xt_buf, stage, wqkv, wot, w1, w3, w2t, res, nrm, mem, o_buf, h_buf, ff_main, ff_tail,
            fill1, fill2, sem_x, sem_qkv, sem_o, sem_ff, sem_out,
            *, seg, n_mem, n_heads, head_dim):
    d_model, seq = xt_buf.shape
    d_ff = w1.shape[1]
    d_main = d_model // LANES * LANES
    n_seg = seq // seg
    n_pairs = n_heads // 2
    n_groups = n_heads // HEAD_GROUP
    n_chunks = d_ff // FF_CHUNK
    score_scale = head_dim ** -0.5 * LOG2E
    head_cols = 3 * head_dim

    x_copy = pltpu.make_async_copy(xt_hbm, xt_buf, sem_x)

    def qkv_copy(pair, which):
        src = (wq_hbm, wk_hbm, wv_hbm)[which].bitcast(jnp.uint32)
        return pltpu.make_async_copy(src.at[:, pair, :], stage.at[which, pair],
                                     sem_qkv.at[which, pair])

    def wo_copy(head):
        return pltpu.make_async_copy(wot_hbm.bitcast(jnp.uint32).at[head],
                                     wot.at[:, pl.ds(head * head_dim, head_dim)], sem_o.at[head])

    ff_copies = [pltpu.make_async_copy(src.bitcast(jnp.uint32), dst, sem_ff.at[i])
                 for i, (src, dst) in enumerate(((w1_hbm, w1), (w3_hbm, w3), (w2t_hbm, w2t)))]

    x_copy.start()
    for pair in range(COPY_WINDOW):
        for which in range(3):
            qkv_copy(pair, which).start()

    fill1[...] = _mask_fill(1, seg, n_mem)
    fill2[...] = _mask_fill(2, seg, n_mem)
    mem0 = mem0_ref[...].astype(F32)
    mem[0:n_mem, :] = mem0
    mem[n_mem:2 * n_mem, :] = mem0

    res[seq:, :] = jnp.zeros((4 * seg, d_model), F32)
    ff_main[...] = jnp.zeros(ff_main.shape, F32)
    ff_tail[...] = jnp.zeros(ff_tail.shape, F32)

    x_copy.wait()

    def load_tokens(j, carry):
        tok = pl.ds(pl.multiple_of(j * LANES, LANES), LANES)
        x = xt_buf[:, tok].astype(F32).T
        res[tok, :] = x
        nrm[tok, :] = _layernorm(x).astype(BF16)
        return carry

    lax.fori_loop(0, seq // LANES, load_tokens, 0)

    def unpack_pair(pair, carry):
        @pl.when(pair + COPY_WINDOW < n_pairs)
        def _():
            for which in range(3):
                qkv_copy(pair + COPY_WINDOW, which).start()

        @pl.when(pair + COPY_WINDOW == n_pairs)
        def _():
            for head in range(n_heads):
                wo_copy(head).start()

        for which in range(3):
            qkv_copy(pair, which).wait()
            words = stage[which, pair]
            even = lax.bitcast_convert_type(words << 16, F32)
            odd = lax.bitcast_convert_type(words & jnp.uint32(0xFFFF0000), F32)
            for parity, w in enumerate((even, odd)):
                col = (2 * pair + parity) * head_cols + which * head_dim
                wqkv[:, pl.ds(pl.multiple_of(col, LANES), head_dim)] = pltpu.bitcast(
                    w.astype(BF16), jnp.uint32)
        return carry

    lax.fori_loop(0, n_pairs, unpack_pair, 0)
    for head in range(n_heads):
        wo_copy(head).wait()
    for copy in ff_copies:
        copy.start()

    def seg_rows(s):
        return pl.ds(pl.multiple_of(s * seg, seg), seg)

    def add_and_normalize(s, delta):
        x = res[seg_rows(s), :] + delta
        normalized = _layernorm(x).astype(BF16)
        res[seg_rows(s), :] = x
        nrm[seg_rows(s), :] = normalized
        return normalized

    def attention_stages(h, fill_ref):
        rows = h.shape[0]
        qkv, probs = {}, {}
        for g in range(n_groups + 2):
            if g < n_groups:
                cols = slice(g * HEAD_GROUP * head_cols, (g + 1) * HEAD_GROUP * head_cols)
                qkv[g] = _dot(h, _as_bf16(wqkv[:, cols])).astype(BF16)
            if 0 <= g - 1 < n_groups:
                y = qkv[g - 1]
                probs[g - 1] = []
                for i in range(HEAD_GROUP):
                    q = y[:, i * head_cols:i * head_cols + head_dim]
                    k = y[:, i * head_cols + head_dim:i * head_cols + 2 * head_dim]
                    fill = fill_ref[...]
                    s = jnp.where(fill == 0.0, _dot_nt(q, k) * score_scale, fill)
                    e = jnp.exp2(s - jnp.max(s, axis=-1, keepdims=True))
                    p = e * (1.0 / jnp.sum(e, axis=-1, keepdims=True))
                    probs[g - 1].append(p.astype(BF16))
            if 0 <= g - 2 < n_groups:
                y = qkv.pop(g - 2)
                for i, p in enumerate(probs.pop(g - 2)):
                    v = y[:, i * head_cols + 2 * head_dim:(i + 1) * head_cols]
                    head = (g - 2) * HEAD_GROUP + i
                    o_buf[0:rows, head * head_dim:(head + 1) * head_dim] = _dot(p, v).astype(BF16)
            yield

    def project_main(act, wt_ref):
        return _dot_nt(act, _as_bf16(wt_ref[0:d_main // 2, :]))

    def project_tail(act, wt_ref):
        return _dot_nt(_as_bf16(wt_ref[d_main // 2:, :]), act)

    def gate_up(hf, c, rows):
        cols = slice(c * FF_CHUNK, (c + 1) * FF_CHUNK)
        gate = _dot(hf, _as_bf16(w1[:, cols]))
        up = _dot(hf, _as_bf16(w3[:, cols]))
        h_buf[rows, cols] = (gate * (1.0 / (1.0 + jnp.exp(-gate))) * up).astype(BF16)

    def ff_input(t):
        sa, sb = ff_blocks(t)
        return jnp.concatenate([nrm[seg_rows(sa), :], nrm[seg_rows(sb), :]], axis=0)

    def ff_finish(segments):
        out = jnp.concatenate([ff_main[...], ff_tail[...].T], axis=1)
        for i, s in enumerate(segments):
            add_and_normalize(s, out[i * seg:(i + 1) * seg, :])

    def ff_blocks(t):
        head = t <= LAG
        tail = t > n_seg
        sa = jnp.where(head, 2 * (t - LAG // 2 - 1), jnp.where(tail, t - LAG - 2, t - 1))
        sb = jnp.where(head | tail, sa + 1, t - LAG - 1)
        return sa, sb

    first_ff = LAG // 2 + 1

    def has_ff(t):
        in_tail = (t > n_seg) & ((t - n_seg) % 2 == 0)
        return ((t >= first_ff) & (t <= n_seg)) | in_tail

    def fused_pair(i, carry):
        t = LAG + 2 * i
        tokens = [[nrm[seg_rows(t + j), :], nrm[seg_rows(t + j - LAG), :]] for j in range(2)]
        ff_in = ff_input(t)
        pending = ff_blocks(t - 2) + ff_blocks(t - 1)
        ff_finish([jnp.where(i == 0, n_seg + j, s) for j, s in enumerate(pending)])
        memory = mem[...]
        for j in range(2):
            ff_rows = slice(2 * j * seg, 2 * (j + 1) * seg)
            h = jnp.concatenate(tokens[j] + [memory.astype(BF16)], axis=0)
            chunk = 0
            for g, _ in enumerate(attention_stages(h, fill2)):
                if g >= n_groups - 1:
                    gate_up(ff_in, chunk, ff_rows)
                    chunk += 1
            for c in range(chunk, n_chunks):
                gate_up(ff_in, c, ff_rows)
            heads = o_buf[...]
            tail = project_tail(heads, wot)
            out = jnp.concatenate([project_main(heads, wot), tail.T], axis=1)
            if j == 1:
                ff_tail[...] = project_tail(h_buf[...], w2t)
            ff_main[ff_rows, :] = project_main(h_buf[ff_rows, :], w2t)
            memory = out[2 * seg:, :]
            ff_in = jnp.concatenate([add_and_normalize(t + j, out[0:seg, :]),
                                     add_and_normalize(t + j - LAG, out[seg:2 * seg, :])], axis=0)
        mem[...] = memory
        return carry

    def edge_step(t, carry):
        @pl.when(t == first_ff)
        def _():
            for copy in ff_copies:
                copy.wait()

        @pl.when(t == LAG)
        def _():
            lax.fori_loop(0, (n_seg - LAG) // 2, fused_pair, 0)
            ff_finish(ff_blocks(n_seg - 2) + ff_blocks(n_seg - 1))

        t = jnp.where(t >= LAG, t + n_seg - LAG, t)

        @pl.when(t < n_seg + LAG)
        def _():
            second = t >= n_seg
            s = jnp.where(second, t - LAG, t)
            mem_rows = pl.ds(pl.multiple_of(jnp.where(second, n_mem, 0), n_mem), n_mem)
            h = jnp.concatenate(
                [nrm[seg_rows(s), :].astype(F32), mem[mem_rows, :]], axis=0).astype(BF16)
            for _ in attention_stages(h, fill1):
                pass
            out = _dot_nt(o_buf[0:seg + n_mem, :], _as_bf16(wot[...]))
            mem[mem_rows, :] = out[seg:, :]
            add_and_normalize(s, out[0:seg, :])

        @pl.when(has_ff(t))
        def _():
            hf = ff_input(t)
            for c in range(n_chunks):
                gate_up(hf, c, slice(0, 2 * seg))
            out = _dot_nt(h_buf[0:2 * seg, :], _as_bf16(w2t[...]))
            for i, s in enumerate(ff_blocks(t)):
                add_and_normalize(s, out[i * seg:(i + 1) * seg, :])

        return carry

    lax.fori_loop(0, 2 * LAG + 1, edge_step, 0)

    def out_copy(j):
        tok = pl.ds(pl.multiple_of(j * LANES, LANES), LANES)
        return pltpu.make_async_copy(xt_buf.at[:, tok], out_hbm.at[:, tok], sem_out.at[j])

    def store_tokens(j, carry):
        tok = pl.ds(pl.multiple_of(j * LANES, LANES), LANES)
        xt_buf[:, tok] = res[tok, :].T.astype(BF16)
        out_copy(j).start()
        return carry

    lax.fori_loop(0, seq // LANES, store_tokens, 0)

    def wait_tokens(j, carry):
        out_copy(j).wait()
        return carry

    lax.fori_loop(0, seq // LANES, wait_tokens, 0)


@functools.partial(jax.jit, static_argnames=("A_seg_len",))
def pallas_interleave_layers__memory_aug_recurrent_mem_tr__glu_gated_swiglu__prompt_kernel(
    A_x: jax.Array,
    A_mem0: jax.Array,
    A_Wq: jax.Array,
    A_Wk: jax.Array,
    A_Wv: jax.Array,
    A_Wo: jax.Array,
    A_seg_len: int,
    B_x: jax.Array,
    B_w1: jax.Array,
    B_w3: jax.Array,
    B_w2: jax.Array,
):
    del B_x
    batch, seq, d_model = A_x.shape
    n_mem = A_mem0.shape[1]
    _, n_heads, head_dim = A_Wq.shape
    d_ff = B_w1.shape[1]
    seg = int(A_seg_len)
    assert batch == 1 and seq % LANES == 0 and seq % seg == 0 and head_dim == LANES
    assert d_ff % FF_CHUNK == 0 and n_heads % HEAD_GROUP == 0 and LAG % 2 == 0
    rows = 2 * (seg + n_mem)

    any_spec = pl.BlockSpec(memory_space=pl.ANY)
    out_t = pl.pallas_call(
        functools.partial(_kernel, seg=seg, n_mem=n_mem, n_heads=n_heads, head_dim=head_dim),
        out_shape=jax.ShapeDtypeStruct((d_model, seq), A_x.dtype),
        in_specs=[any_spec, pl.BlockSpec(memory_space=pltpu.VMEM)] + [any_spec] * 7,
        out_specs=any_spec,
        scratch_shapes=[
            pltpu.VMEM((d_model, seq), BF16),
            pltpu.VMEM((3, n_heads // 2, d_model, head_dim), jnp.uint32),
            pltpu.VMEM((d_model // 2, 3 * n_heads * head_dim), jnp.uint32),
            pltpu.VMEM((d_model // 2, n_heads * head_dim), jnp.uint32),
            pltpu.VMEM((d_model // 2, d_ff), jnp.uint32),
            pltpu.VMEM((d_model // 2, d_ff), jnp.uint32),
            pltpu.VMEM((d_model // 2, d_ff), jnp.uint32),
            pltpu.VMEM((seq + 4 * seg, d_model), F32),
            pltpu.VMEM((seq + 4 * seg, d_model), BF16),
            pltpu.VMEM((2 * n_mem, d_model), F32),
            pltpu.VMEM((rows, n_heads * head_dim), BF16),
            pltpu.VMEM((4 * seg, d_ff), BF16),
            pltpu.VMEM((4 * seg, d_model // LANES * LANES), F32),
            pltpu.VMEM((d_model % LANES, 4 * seg), F32),
            pltpu.VMEM((rows // 2, rows // 2), F32),
            pltpu.VMEM((rows, rows), F32),
            pltpu.SemaphoreType.DMA(()),
            pltpu.SemaphoreType.DMA((3, n_heads // 2)),
            pltpu.SemaphoreType.DMA((n_heads,)),
            pltpu.SemaphoreType.DMA((3,)),
            pltpu.SemaphoreType.DMA((seq // LANES,)),
        ],
        compiler_params=pltpu.CompilerParams(vmem_limit_bytes=100 * 1024 * 1024),
    )(
        A_x[0].T,
        A_mem0[0],
        A_Wq,
        A_Wk,
        A_Wv,
        jnp.transpose(A_Wo, (0, 2, 1)),
        B_w1,
        B_w3,
        B_w2.T,
    )
    return out_t.T[None]
```

```python
import functools
import math

import jax
import jax.numpy as jnp
from jax import lax
import jax.experimental.pallas as pl
import jax.experimental.pallas.tpu as pltpu

F32 = jnp.float32
BF16 = jnp.bfloat16
LANES = 128
LAG = 4
HEAD_GROUP = 2
EDGE_GROUP = 4
N_EARLY = 10
FF_CHUNK = 512
COPY_WINDOW = 2
LN_EPS = 1e-5
MASK_FILL = -1000000000.0
LOG2E = math.log2(math.e)
NT_DIMS = (((1,), (1,)), ((), ()))


def _dot(a, b):
    return jnp.dot(a, b, preferred_element_type=F32)


def _dot_nt(a, b):
    return lax.dot_general(a, b, NT_DIMS, preferred_element_type=F32)


def _as_bf16(words):
    return pltpu.bitcast(words, BF16)


def _layernorm(x):
    mean = jnp.mean(x, axis=-1, keepdims=True)
    cen = x - mean
    var = jnp.mean(cen * cen, axis=-1, keepdims=True)
    return cen * lax.rsqrt(var + LN_EPS)


def _mask_fill(n_streams, seg, n_mem):
    rows = n_streams * (seg + n_mem)

    def stream_and_pos(i):
        is_mem = i >= n_streams * seg
        j = i - n_streams * seg
        stream = jnp.where(is_mem, j // n_mem, i // seg)
        pos = jnp.where(is_mem, j % n_mem, n_mem + i % seg)
        return stream, pos

    q_stream, q_pos = stream_and_pos(lax.broadcasted_iota(jnp.int32, (rows, rows), 0))
    k_stream, k_pos = stream_and_pos(lax.broadcasted_iota(jnp.int32, (rows, rows), 1))
    visible = (q_pos < n_mem) | (q_pos >= k_pos)
    fill = jnp.where(visible, 0.0, MASK_FILL * LOG2E).astype(F32)
    return jnp.where(q_stream == k_stream, fill, -jnp.inf)


def _kernel(xt_hbm, mem0_ref, wq_hbm, wk_hbm, wv_hbm, wot_hbm, w1_hbm, w3_hbm, w2t_hbm,
            out_hbm,
            xt_buf, stage, early, wqkv, wot, w1, w3, w2t, res, nrm, mem, o_buf, h_buf, ff_main, ff_tail,
            fill1, fill2, sem_x, sem_qkv, sem_o, sem_ff, sem_out,
            *, seg, n_mem, n_heads, head_dim):
    d_model, seq = xt_buf.shape
    d_ff = w1.shape[1]
    d_main = d_model // LANES * LANES
    n_seg = seq // seg
    n_pairs = n_heads // 2
    n_chunks = d_ff // FF_CHUNK
    score_scale = head_dim ** -0.5 * LOG2E
    head_cols = 3 * head_dim

    x_copy = pltpu.make_async_copy(xt_hbm, xt_buf, sem_x)

    def qkv_copy(pair, which):
        src = (wq_hbm, wk_hbm, wv_hbm)[which].bitcast(jnp.uint32)
        return pltpu.make_async_copy(src.at[:, pair, :], stage.at[which, pair],
                                     sem_qkv.at[which, pair])

    def wo_copy(head):
        return pltpu.make_async_copy(wot_hbm.bitcast(jnp.uint32).at[head],
                                     wot.at[:, pl.ds(head * head_dim, head_dim)], sem_o.at[head])

    ff_copies = [pltpu.make_async_copy(src.bitcast(jnp.uint32), dst, sem_ff.at[i])
                 for i, (src, dst) in enumerate(((w1_hbm, w1), (w3_hbm, w3), (w2t_hbm, w2t)))]

    x_copy.start()
    for pair in range(COPY_WINDOW):
        for which in range(3):
            qkv_copy(pair, which).start()

    fill1[...] = _mask_fill(1, seg, n_mem)
    fill2[...] = _mask_fill(2, seg, n_mem)
    mem0 = mem0_ref[...].astype(F32)
    mem[0:n_mem, :] = mem0
    mem[n_mem:2 * n_mem, :] = mem0

    ff_main[...] = jnp.zeros(ff_main.shape, F32)
    ff_tail[...] = jnp.zeros(ff_tail.shape, F32)

    x_copy.wait()

    for pair in range(COPY_WINDOW, 2 * COPY_WINDOW):
        for which in range(3):
            qkv_copy(pair, which).start()

    def load_tokens(src_block, dst_block):
        x = xt_buf[:, pl.ds(pl.multiple_of(src_block * LANES, LANES), LANES)].astype(F32).T
        rows = pl.ds(pl.multiple_of(dst_block * LANES, LANES), LANES)
        res[rows, :] = x
        nrm[rows, :] = _layernorm(x).astype(BF16)

    n_blocks = seq // LANES
    first_early = n_seg - N_EARLY
    late_blocks = first_early * seg // LANES

    def load_early(j, carry):
        load_tokens(j, j)
        return carry

    lax.fori_loop(late_blocks, n_blocks, load_early, 0)

    def prepare_pair(pair, carry):
        ahead = pair + 2 * COPY_WINDOW

        @pl.when(ahead < n_pairs)
        def _():
            for which in range(3):
                qkv_copy(ahead, which).start()

        @pl.when(ahead == n_pairs)
        def _():
            for head in range(n_heads):
                wo_copy(head).start()

        for which in range(3):
            qkv_copy(pair, which).wait()
        words = [stage[which, pair] for which in range(3)]
        even = [lax.bitcast_convert_type(w << 16, F32) for w in words]
        odd = [lax.bitcast_convert_type(w & jnp.uint32(0xFFFF0000), F32) for w in words]
        w_pair = jnp.concatenate([w.astype(BF16) for w in even + odd], axis=1)
        cols = pl.ds(pl.multiple_of(pair * 2 * head_cols, LANES), 2 * head_cols)
        early[:, cols] = _dot(nrm[first_early * seg:seq, :], w_pair).astype(BF16)
        wqkv[:, cols] = pltpu.bitcast(w_pair, jnp.uint32)

        spare = pair >= late_blocks
        load_tokens(jnp.where(spare, 0, pair), jnp.where(spare, n_blocks, pair))
        return carry

    lax.fori_loop(0, n_pairs, prepare_pair, 0)
    for head in range(n_heads):
        wo_copy(head).wait()
    for copy in ff_copies:
        copy.start()

    def seg_rows(s):
        start = s * seg if isinstance(s, int) else pl.multiple_of(s * seg, seg)
        return pl.ds(start, seg)

    def add_and_normalize(s, delta):
        x = res[seg_rows(s), :] + delta
        normalized = _layernorm(x).astype(BF16)
        res[seg_rows(s), :] = x
        nrm[seg_rows(s), :] = normalized
        return normalized

    def attention_stages(h, fill_ref, group, early_rows=None):
        rows = fill_ref.shape[0]
        n_groups = n_heads // group
        qkv, probs = {}, {}
        for g in range(n_groups + 2):
            if g < n_groups:
                cols = slice(g * group * head_cols, (g + 1) * group * head_cols)
                qkv[g] = _dot(h, _as_bf16(wqkv[:, cols])).astype(BF16)
                if early_rows is not None:
                    qkv[g] = jnp.concatenate([early[early_rows, cols], qkv[g]], axis=0)
            if 0 <= g - 1 < n_groups:
                y = qkv[g - 1]
                probs[g - 1] = []
                for i in range(group):
                    q = y[:, i * head_cols:i * head_cols + head_dim]
                    k = y[:, i * head_cols + head_dim:i * head_cols + 2 * head_dim]
                    fill = fill_ref[...]
                    s = jnp.where(fill == 0.0, _dot_nt(q, k) * score_scale, fill)
                    e = jnp.exp2(s - jnp.max(s, axis=-1, keepdims=True))
                    p = e * (1.0 / jnp.sum(e, axis=-1, keepdims=True))
                    probs[g - 1].append(p.astype(BF16))
            if 0 <= g - 2 < n_groups:
                y = qkv.pop(g - 2)
                for i, p in enumerate(probs.pop(g - 2)):
                    v = y[:, i * head_cols + 2 * head_dim:(i + 1) * head_cols]
                    head = (g - 2) * group + i
                    o_buf[0:rows, head * head_dim:(head + 1) * head_dim] = _dot(p, v).astype(BF16)
            yield g >= n_groups - 1

    def project_main(act, wt_ref):
        return _dot_nt(act, _as_bf16(wt_ref[0:d_main // 2, :]))

    def project_tail(act, wt_ref):
        return _dot_nt(_as_bf16(wt_ref[d_main // 2:, :]), act)

    def gate_up(hf, c, rows):
        cols = slice(c * FF_CHUNK, (c + 1) * FF_CHUNK)
        gate = _dot(hf, _as_bf16(w1[:, cols]))
        up = _dot(hf, _as_bf16(w3[:, cols]))
        h_buf[rows, cols] = (gate * (1.0 / (1.0 + jnp.exp(-gate))) * up).astype(BF16)

    def ff_input(t):
        sa, sb = ff_blocks(t)
        return jnp.concatenate([nrm[seg_rows(sa), :], nrm[seg_rows(sb), :]], axis=0)

    def ff_finish(segments):
        out = jnp.concatenate([ff_main[...], ff_tail[...].T], axis=1)
        for i, s in enumerate(segments):
            add_and_normalize(s, out[i * seg:(i + 1) * seg, :])

    def ff_blocks(t):
        if isinstance(t, int):
            return t - 1, t - LAG - 1
        return t - 1, jnp.where(t == LAG, t - 2, t - LAG - 1)

    def fused_step(t, stages, ff_in, ff_rows, with_tail, lead=0):
        chunks = iter(range(n_chunks))
        for _ in range(lead):
            gate_up(ff_in, next(chunks), ff_rows)
        for draining in stages:
            if draining:
                gate_up(ff_in, next(chunks), ff_rows)
        for c in chunks:
            gate_up(ff_in, c, ff_rows)
        heads = o_buf[...]
        tail = project_tail(heads, wot)
        out = jnp.concatenate([project_main(heads, wot), tail.T], axis=1)
        if with_tail:
            ff_tail[...] = project_tail(h_buf[...], w2t)
        ff_main[ff_rows, :] = project_main(h_buf[ff_rows, :], w2t)
        next_in = jnp.concatenate([add_and_normalize(t, out[0:seg, :]),
                                   add_and_normalize(t - LAG, out[seg:2 * seg, :])], axis=0)
        return out[2 * seg:, :], next_in

    def early_step(t, carry):
        odd = t % 2

        @pl.when(odd == 0)
        def _():
            ff_finish(ff_blocks(t - 2) + ff_blocks(t - 1))

        h = jnp.concatenate([nrm[seg_rows(t - LAG), :], mem[...].astype(BF16)], axis=0)
        stages = attention_stages(h, fill2, HEAD_GROUP, seg_rows(t - first_early))
        ff_rows = pl.ds(pl.multiple_of(odd * 2 * seg, 2 * seg), 2 * seg)
        mem[...], _ = fused_step(t, stages, ff_input(t), ff_rows, with_tail=False)

        @pl.when(odd == 1)
        def _():
            ff_tail[...] = project_tail(h_buf[...], w2t)

        return carry

    def fused_pair(i, carry):
        t = LAG + 2 * i
        ff_in = ff_input(t)
        pending = ff_blocks(t - 2) + ff_blocks(t - 1)
        ff_finish([jnp.where(i == 0, n_seg + j, s) for j, s in enumerate(pending)])
        memory = mem[...]
        for j in range(2):
            h = jnp.concatenate([nrm[seg_rows(t + j), :], nrm[seg_rows(t + j - LAG), :],
                                 memory.astype(BF16)], axis=0)
            memory, ff_in = fused_step(t + j, attention_stages(h, fill2, HEAD_GROUP), ff_in,
                                       slice(2 * j * seg, 2 * (j + 1) * seg),
                                       with_tail=j == 1, lead=1 - j)
        mem[...] = memory
        return carry

    def single_attention(s, layer):
        mem_rows = slice(layer * n_mem, (layer + 1) * n_mem)
        h = jnp.concatenate(
            [nrm[seg_rows(s), :].astype(F32), mem[mem_rows, :]], axis=0).astype(BF16)
        for _ in attention_stages(h, fill1, EDGE_GROUP):
            pass
        out = _dot_nt(o_buf[0:seg + n_mem, :], _as_bf16(wot[...]))
        mem[mem_rows, :] = out[seg:, :]
        add_and_normalize(s, out[0:seg, :])

    def single_ff(s):
        hf = jnp.concatenate([nrm[seg_rows(s + i), :] for i in range(2)], axis=0)
        for c in range(n_chunks):
            gate_up(hf, c, slice(0, 2 * seg))
        out = _dot_nt(h_buf[0:2 * seg, :], _as_bf16(w2t[...]))
        for i in range(2):
            add_and_normalize(s + i, out[i * seg:(i + 1) * seg, :])

    def head_step(s, carry):
        single_attention(s, 0)
        return carry

    def tail_step(s, carry):
        single_attention(s, 1)

        @pl.when(s % 2 == 1)
        def _():
            single_ff(s - 1)

        return carry

    lax.fori_loop(0, LAG, head_step, 0)
    for copy in ff_copies:
        copy.wait()
    single_ff(0)
    lax.fori_loop(0, (first_early - LAG) // 2, fused_pair, 0)
    lax.fori_loop(first_early, n_seg, early_step, 0)
    ff_finish(ff_blocks(n_seg - 2) + ff_blocks(n_seg - 1))
    last = ff_input(n_seg)
    for c in range(n_chunks):
        gate_up(last, c, slice(0, 2 * seg))
    out = _dot_nt(h_buf[0:2 * seg, :], _as_bf16(w2t[...]))
    for i, s in enumerate(ff_blocks(n_seg)):
        add_and_normalize(s, out[i * seg:(i + 1) * seg, :])
    lax.fori_loop(n_seg - LAG, n_seg, tail_step, 0)

    def out_copy(j):
        tok = pl.ds(pl.multiple_of(j * LANES, LANES), LANES)
        return pltpu.make_async_copy(xt_buf.at[:, tok], out_hbm.at[:, tok], sem_out.at[j])

    def store_tokens(j, carry):
        tok = pl.ds(pl.multiple_of(j * LANES, LANES), LANES)
        xt_buf[:, tok] = res[tok, :].T.astype(BF16)
        out_copy(j).start()
        return carry

    lax.fori_loop(0, seq // LANES, store_tokens, 0)

    def wait_tokens(j, carry):
        out_copy(j).wait()
        return carry

    lax.fori_loop(0, seq // LANES, wait_tokens, 0)


@functools.partial(jax.jit, static_argnames=("A_seg_len",))
def pallas_interleave_layers__memory_aug_recurrent_mem_tr__glu_gated_swiglu__prompt_kernel(
    A_x: jax.Array,
    A_mem0: jax.Array,
    A_Wq: jax.Array,
    A_Wk: jax.Array,
    A_Wv: jax.Array,
    A_Wo: jax.Array,
    A_seg_len: int,
    B_x: jax.Array,
    B_w1: jax.Array,
    B_w3: jax.Array,
    B_w2: jax.Array,
):
    del B_x
    batch, seq, d_model = A_x.shape
    n_mem = A_mem0.shape[1]
    _, n_heads, head_dim = A_Wq.shape
    d_ff = B_w1.shape[1]
    seg = int(A_seg_len)
    assert batch == 1 and seq % LANES == 0 and seq % seg == 0 and head_dim == LANES
    assert d_ff % FF_CHUNK == 0 and n_heads % HEAD_GROUP == 0 and N_EARLY % 2 == 0
    rows = 2 * (seg + n_mem)

    any_spec = pl.BlockSpec(memory_space=pl.ANY)
    out_t = pl.pallas_call(
        functools.partial(_kernel, seg=seg, n_mem=n_mem, n_heads=n_heads, head_dim=head_dim),
        out_shape=jax.ShapeDtypeStruct((d_model, seq), A_x.dtype),
        in_specs=[any_spec, pl.BlockSpec(memory_space=pltpu.VMEM)] + [any_spec] * 7,
        out_specs=any_spec,
        scratch_shapes=[
            pltpu.VMEM((d_model, seq), BF16),
            pltpu.VMEM((3, n_heads // 2, d_model, head_dim), jnp.uint32),
            pltpu.VMEM((N_EARLY * seg, 3 * n_heads * head_dim), BF16),
            pltpu.VMEM((d_model // 2, 3 * n_heads * head_dim), jnp.uint32),
            pltpu.VMEM((d_model // 2, n_heads * head_dim), jnp.uint32),
            pltpu.VMEM((d_model // 2, d_ff), jnp.uint32),
            pltpu.VMEM((d_model // 2, d_ff), jnp.uint32),
            pltpu.VMEM((d_model // 2, d_ff), jnp.uint32),
            pltpu.VMEM((seq + 4 * seg, d_model), F32),
            pltpu.VMEM((seq + 4 * seg, d_model), BF16),
            pltpu.VMEM((2 * n_mem, d_model), F32),
            pltpu.VMEM((rows, n_heads * head_dim), BF16),
            pltpu.VMEM((4 * seg, d_ff), BF16),
            pltpu.VMEM((4 * seg, d_model // LANES * LANES), F32),
            pltpu.VMEM((d_model % LANES, 4 * seg), F32),
            pltpu.VMEM((rows // 2, rows // 2), F32),
            pltpu.VMEM((rows, rows), F32),
            pltpu.SemaphoreType.DMA(()),
            pltpu.SemaphoreType.DMA((3, n_heads // 2)),
            pltpu.SemaphoreType.DMA((n_heads,)),
            pltpu.SemaphoreType.DMA((3,)),
            pltpu.SemaphoreType.DMA((seq // LANES,)),
        ],
        compiler_params=pltpu.CompilerParams(vmem_limit_bytes=100 * 1024 * 1024),
    )(
        A_x[0].T,
        A_mem0[0],
        A_Wq,
        A_Wk,
        A_Wv,
        jnp.transpose(A_Wo, (0, 2, 1)),
        B_w1,
        B_w3,
        B_w2.T,
    )
    return out_t.T[None]
```

```python
import functools
import math

import jax
import jax.numpy as jnp
from jax import lax
import jax.experimental.pallas as pl
import jax.experimental.pallas.tpu as pltpu

F32 = jnp.float32
BF16 = jnp.bfloat16
LANES = 128
LAG = 4
HEAD_GROUP = 2
EDGE_GROUP = 4
N_EARLY = 10
FF_CHUNK = 512
COPY_WINDOW = 2
LN_EPS = 1e-5
MASK_FILL = -1000000000.0
LOG2E = math.log2(math.e)
NT_DIMS = (((1,), (1,)), ((), ()))


def _dot(a, b):
    return jnp.dot(a, b, preferred_element_type=F32)


def _dot_nt(a, b):
    return lax.dot_general(a, b, NT_DIMS, preferred_element_type=F32)


def _as_bf16(words):
    return pltpu.bitcast(words, BF16)


def _block(index, size):
    start = index * size
    return pl.ds(start if isinstance(index, int) else pl.multiple_of(start, size), size)


def _layernorm(x):
    mean = jnp.mean(x, axis=-1, keepdims=True)
    cen = x - mean
    var = jnp.mean(cen * cen, axis=-1, keepdims=True)
    return cen * lax.rsqrt(var + LN_EPS)


def _mask_fill(n_streams, seg, n_mem):
    rows = n_streams * (seg + n_mem)

    def stream_and_pos(i):
        is_mem = i >= n_streams * seg
        j = i - n_streams * seg
        stream = jnp.where(is_mem, j // n_mem, i // seg)
        pos = jnp.where(is_mem, j % n_mem, n_mem + i % seg)
        return stream, pos

    q_stream, q_pos = stream_and_pos(lax.broadcasted_iota(jnp.int32, (rows, rows), 0))
    k_stream, k_pos = stream_and_pos(lax.broadcasted_iota(jnp.int32, (rows, rows), 1))
    visible = (q_pos < n_mem) | (q_pos >= k_pos)
    fill = jnp.where(visible, 0.0, MASK_FILL * LOG2E).astype(F32)
    return jnp.where(q_stream == k_stream, fill, -jnp.inf)


def _kernel(xt_hbm, mem0_ref, wq_hbm, wk_hbm, wv_hbm, wot_hbm, w1_hbm, w3_hbm, w2t_hbm,
            out_hbm,
            xt_buf, stage, early, wqkv, wot, w1, w3, w2t, res, nrm, mem, o_buf, h_buf, ff_main, ff_tail,
            fill1, fill2, sem_x, sem_qkv, sem_o, sem_ff, sem_out,
            *, seg, n_mem, n_heads, head_dim):
    d_model, seq = xt_buf.shape
    d_ff = w1.shape[1]
    d_main = d_model // LANES * LANES
    n_seg = seq // seg
    n_pairs = n_heads // 2
    n_chunks = d_ff // FF_CHUNK
    score_scale = head_dim ** -0.5 * LOG2E
    head_cols = 3 * head_dim

    x_copy = pltpu.make_async_copy(xt_hbm, xt_buf, sem_x)

    def qkv_copy(pair, which):
        src = (wq_hbm, wk_hbm, wv_hbm)[which].bitcast(jnp.uint32)
        return pltpu.make_async_copy(src.at[:, pair, :], stage.at[which, pair],
                                     sem_qkv.at[which, pair])

    def wo_copy(head):
        return pltpu.make_async_copy(wot_hbm.bitcast(jnp.uint32).at[head],
                                     wot.at[:, pl.ds(head * head_dim, head_dim)], sem_o.at[head])

    ff_copies = [pltpu.make_async_copy(src.bitcast(jnp.uint32), dst, sem_ff.at[i])
                 for i, (src, dst) in enumerate(((w1_hbm, w1), (w3_hbm, w3), (w2t_hbm, w2t)))]

    x_copy.start()
    for pair in range(COPY_WINDOW):
        for which in range(3):
            qkv_copy(pair, which).start()

    fill1[...] = _mask_fill(1, seg, n_mem)
    fill2[...] = _mask_fill(2, seg, n_mem)
    mem0 = mem0_ref[...].astype(F32)
    mem[0:n_mem, :] = mem0
    mem[n_mem:2 * n_mem, :] = mem0

    ff_main[...] = jnp.zeros(ff_main.shape, F32)
    ff_tail[...] = jnp.zeros(ff_tail.shape, F32)

    x_copy.wait()

    for pair in range(COPY_WINDOW, 2 * COPY_WINDOW):
        for which in range(3):
            qkv_copy(pair, which).start()

    def load_tokens(src_block, dst_block):
        x = xt_buf[:, _block(src_block, LANES)].astype(F32).T
        rows = _block(dst_block, LANES)
        res[rows, :] = x
        nrm[rows, :] = _layernorm(x).astype(BF16)

    n_blocks = seq // LANES
    first_early = n_seg - N_EARLY
    late_blocks = first_early * seg // LANES

    for block in range(late_blocks, n_blocks):
        load_tokens(block, block)

    def prepare_pair(pair, carry):
        ahead = pair + 2 * COPY_WINDOW

        @pl.when(ahead < n_pairs)
        def _():
            for which in range(3):
                qkv_copy(ahead, which).start()

        @pl.when(ahead == n_pairs)
        def _():
            for head in range(n_heads):
                wo_copy(head).start()

        for which in range(3):
            qkv_copy(pair, which).wait()
        words = [stage[which, pair] for which in range(3)]
        even = [lax.bitcast_convert_type(w << 16, F32) for w in words]
        odd = [lax.bitcast_convert_type(w & jnp.uint32(0xFFFF0000), F32) for w in words]
        w_pair = jnp.concatenate([w.astype(BF16) for w in even + odd], axis=1)
        cols = _block(pair, 2 * head_cols)
        early[:, cols] = _dot(nrm[first_early * seg:seq, :], w_pair).astype(BF16)
        wqkv[:, cols] = pltpu.bitcast(w_pair, jnp.uint32)

        spare = pair >= late_blocks
        load_tokens(jnp.where(spare, 0, pair), jnp.where(spare, n_blocks, pair))
        return carry

    lax.fori_loop(0, n_pairs, prepare_pair, 0)
    for head in range(n_heads):
        wo_copy(head).wait()
    for copy in ff_copies:
        copy.start()

    def seg_rows(s):
        return _block(s, seg)

    def add_and_normalize(s, delta):
        x = res[seg_rows(s), :] + delta
        normalized = _layernorm(x).astype(BF16)
        res[seg_rows(s), :] = x
        nrm[seg_rows(s), :] = normalized
        return normalized

    def attention_stages(h, fill_ref, group, early_rows=None):
        rows = fill_ref.shape[0]
        n_groups = n_heads // group
        qkv, probs = {}, {}
        for g in range(n_groups + 2):
            if g < n_groups:
                cols = slice(g * group * head_cols, (g + 1) * group * head_cols)
                qkv[g] = _dot(h, _as_bf16(wqkv[:, cols])).astype(BF16)
                if early_rows is not None:
                    qkv[g] = jnp.concatenate([early[early_rows, cols], qkv[g]], axis=0)
            if 0 <= g - 1 < n_groups:
                y = qkv[g - 1]
                probs[g - 1] = []
                for i in range(group):
                    q = y[:, i * head_cols:i * head_cols + head_dim]
                    k = y[:, i * head_cols + head_dim:i * head_cols + 2 * head_dim]
                    fill = fill_ref[...]
                    s = jnp.where(fill == 0.0, _dot_nt(q, k) * score_scale, fill)
                    e = jnp.exp2(s - jnp.max(s, axis=-1, keepdims=True))
                    p = e * (1.0 / jnp.sum(e, axis=-1, keepdims=True))
                    probs[g - 1].append(p.astype(BF16))
            if 0 <= g - 2 < n_groups:
                y = qkv.pop(g - 2)
                for i, p in enumerate(probs.pop(g - 2)):
                    v = y[:, i * head_cols + 2 * head_dim:(i + 1) * head_cols]
                    head = (g - 2) * group + i
                    o_buf[0:rows, head * head_dim:(head + 1) * head_dim] = _dot(p, v).astype(BF16)
            yield g >= n_groups - 1

    def project_main(act, wt_ref):
        return _dot_nt(act, _as_bf16(wt_ref[0:d_main // 2, :]))

    def project_tail(act, wt_ref):
        return _dot_nt(_as_bf16(wt_ref[d_main // 2:, :]), act)

    def gate_up(hf, c, rows):
        cols = slice(c * FF_CHUNK, (c + 1) * FF_CHUNK)
        gate = _dot(hf, _as_bf16(w1[:, cols]))
        up = _dot(hf, _as_bf16(w3[:, cols]))
        h_buf[rows, cols] = (gate * (1.0 / (1.0 + jnp.exp(-gate))) * up).astype(BF16)

    def ff_input(t):
        sa, sb = ff_blocks(t)
        return jnp.concatenate([nrm[seg_rows(sa), :], nrm[seg_rows(sb), :]], axis=0)

    def ff_finish(segments):
        out = jnp.concatenate([ff_main[...], ff_tail[...].T], axis=1)
        for i, s in enumerate(segments):
            add_and_normalize(s, out[i * seg:(i + 1) * seg, :])

    def ff_blocks(t):
        if isinstance(t, int):
            return t - 1, t - LAG - 1
        return t - 1, jnp.where(t == LAG, t - 2, t - LAG - 1)

    def out_copy(block):
        tok = _block(block, LANES)
        return pltpu.make_async_copy(xt_buf.at[:, tok], out_hbm.at[:, tok], sem_out.at[block])

    def stage_output(block):
        tok = _block(block, LANES)
        xt_buf[:, tok] = res[tok, :].T.astype(BF16)

    def fused_step(t, stages, ff_in, ff_rows, with_tail, lead=0):
        chunks = iter(range(n_chunks))
        for _ in range(lead):
            gate_up(ff_in, next(chunks), ff_rows)
        for draining in stages:
            if draining:
                gate_up(ff_in, next(chunks), ff_rows)
        for c in chunks:
            gate_up(ff_in, c, ff_rows)
        heads = o_buf[...]
        tail = project_tail(heads, wot)
        out = jnp.concatenate([project_main(heads, wot), tail.T], axis=1)
        if with_tail:
            ff_tail[...] = project_tail(h_buf[...], w2t)
        ff_main[ff_rows, :] = project_main(h_buf[ff_rows, :], w2t)
        next_in = jnp.concatenate([add_and_normalize(t, out[0:seg, :]),
                                   add_and_normalize(t - LAG, out[seg:2 * seg, :])], axis=0)
        return out[2 * seg:, :], next_in

    def early_step(t, carry):
        odd = t % 2

        @pl.when(odd == 0)
        def _():
            ff_finish(ff_blocks(t - 2) + ff_blocks(t - 1))

        stage_output(t - first_early)
        h = jnp.concatenate([nrm[seg_rows(t - LAG), :], mem[...].astype(BF16)], axis=0)
        stages = attention_stages(h, fill2, HEAD_GROUP, seg_rows(t - first_early))
        ff_rows = _block(odd, 2 * seg)
        mem[...], _ = fused_step(t, stages, ff_input(t), ff_rows, with_tail=False)
        out_copy(t - first_early).start()

        @pl.when(odd == 1)
        def _():
            ff_tail[...] = project_tail(h_buf[...], w2t)

        return carry

    def fused_pair(i, carry):
        t = LAG + 2 * i
        ff_in = ff_input(t)
        pending = ff_blocks(t - 2) + ff_blocks(t - 1)
        ff_finish([jnp.where(i == 0, n_seg + j, s) for j, s in enumerate(pending)])
        memory = mem[...]
        for j in range(2):
            h = jnp.concatenate([nrm[seg_rows(t + j), :], nrm[seg_rows(t + j - LAG), :],
                                 memory.astype(BF16)], axis=0)
            memory, ff_in = fused_step(t + j, attention_stages(h, fill2, HEAD_GROUP), ff_in,
                                       slice(2 * j * seg, 2 * (j + 1) * seg),
                                       with_tail=j == 1, lead=1 - j)
        mem[...] = memory
        return carry

    def edge_step(s=None, layer=None, ff_segments=None):
        ff_rows = slice(0, 2 * seg)
        chunks = iter(range(n_chunks) if ff_segments else ())
        if ff_segments:
            ff_in = jnp.concatenate([nrm[seg_rows(f), :] for f in ff_segments], axis=0)
        if s is not None:
            mem_rows = slice(layer * n_mem, (layer + 1) * n_mem)
            h = jnp.concatenate(
                [nrm[seg_rows(s), :].astype(F32), mem[mem_rows, :]], axis=0).astype(BF16)
            for draining in attention_stages(h, fill1, EDGE_GROUP):
                if draining and ff_segments:
                    gate_up(ff_in, next(chunks), ff_rows)
        for c in chunks:
            gate_up(ff_in, c, ff_rows)
        if s is not None:
            out = _dot_nt(o_buf[0:seg + n_mem, :], _as_bf16(wot[...]))
        if ff_segments:
            ff_out = _dot_nt(h_buf[ff_rows, :], _as_bf16(w2t[...]))
        if s is not None:
            mem[mem_rows, :] = out[seg:, :]
            add_and_normalize(s, out[0:seg, :])
        for i, f in enumerate(ff_segments or ()):
            add_and_normalize(f, ff_out[i * seg:(i + 1) * seg, :])

    def head_step(s, carry):
        edge_step(s, 0)
        return carry

    def tail_pair(i, carry):
        s = n_seg - LAG + 2 * i
        block = N_EARLY + 2 * i
        stage_output(block)
        edge_step(s, 1, (jnp.where(i == 0, n_seg - 1, s - 2), s - 1))
        out_copy(block).start()
        stage_output(block + 1)
        edge_step(s + 1, 1)
        out_copy(block + 1).start()
        return carry

    lax.fori_loop(0, LAG, head_step, 0)
    for copy in ff_copies:
        copy.wait()
    edge_step(ff_segments=(0, 1))
    lax.fori_loop(0, (first_early - LAG) // 2, fused_pair, 0)
    lax.fori_loop(first_early, n_seg, early_step, 0)
    ff_finish(ff_blocks(n_seg - 2) + ff_blocks(n_seg - 1))
    lax.fori_loop(0, LAG // 2, tail_pair, 0)
    edge_step(ff_segments=(n_seg - 2, n_seg - 1))
    for block in range(N_EARLY + LAG, n_blocks):
        stage_output(block)
        out_copy(block).start()
    for block in range(n_blocks):
        out_copy(block).wait()


@functools.partial(jax.jit, static_argnames=("A_seg_len",))
def pallas_interleave_layers__memory_aug_recurrent_mem_tr__glu_gated_swiglu__prompt_kernel(
    A_x: jax.Array,
    A_mem0: jax.Array,
    A_Wq: jax.Array,
    A_Wk: jax.Array,
    A_Wv: jax.Array,
    A_Wo: jax.Array,
    A_seg_len: int,
    B_x: jax.Array,
    B_w1: jax.Array,
    B_w3: jax.Array,
    B_w2: jax.Array,
):
    del B_x
    batch, seq, d_model = A_x.shape
    n_mem = A_mem0.shape[1]
    _, n_heads, head_dim = A_Wq.shape
    d_ff = B_w1.shape[1]
    seg = int(A_seg_len)
    assert batch == 1 and seq % LANES == 0 and seq % seg == 0 and head_dim == LANES
    assert d_ff % FF_CHUNK == 0 and n_heads % HEAD_GROUP == 0 and N_EARLY % 2 == 0 and LAG == 4
    rows = 2 * (seg + n_mem)

    any_spec = pl.BlockSpec(memory_space=pl.ANY)
    out_t = pl.pallas_call(
        functools.partial(_kernel, seg=seg, n_mem=n_mem, n_heads=n_heads, head_dim=head_dim),
        out_shape=jax.ShapeDtypeStruct((d_model, seq), A_x.dtype),
        in_specs=[any_spec, pl.BlockSpec(memory_space=pltpu.VMEM)] + [any_spec] * 7,
        out_specs=any_spec,
        scratch_shapes=[
            pltpu.VMEM((d_model, seq), BF16),
            pltpu.VMEM((3, n_heads // 2, d_model, head_dim), jnp.uint32),
            pltpu.VMEM((N_EARLY * seg, 3 * n_heads * head_dim), BF16),
            pltpu.VMEM((d_model // 2, 3 * n_heads * head_dim), jnp.uint32),
            pltpu.VMEM((d_model // 2, n_heads * head_dim), jnp.uint32),
            pltpu.VMEM((d_model // 2, d_ff), jnp.uint32),
            pltpu.VMEM((d_model // 2, d_ff), jnp.uint32),
            pltpu.VMEM((d_model // 2, d_ff), jnp.uint32),
            pltpu.VMEM((seq + 4 * seg, d_model), F32),
            pltpu.VMEM((seq + 4 * seg, d_model), BF16),
            pltpu.VMEM((2 * n_mem, d_model), F32),
            pltpu.VMEM((rows, n_heads * head_dim), BF16),
            pltpu.VMEM((4 * seg, d_ff), BF16),
            pltpu.VMEM((4 * seg, d_model // LANES * LANES), F32),
            pltpu.VMEM((d_model % LANES, 4 * seg), F32),
            pltpu.VMEM((rows // 2, rows // 2), F32),
            pltpu.VMEM((rows, rows), F32),
            pltpu.SemaphoreType.DMA(()),
            pltpu.SemaphoreType.DMA((3, n_heads // 2)),
            pltpu.SemaphoreType.DMA((n_heads,)),
            pltpu.SemaphoreType.DMA((3,)),
            pltpu.SemaphoreType.DMA((seq // LANES,)),
        ],
        compiler_params=pltpu.CompilerParams(vmem_limit_bytes=100 * 1024 * 1024),
    )(
        A_x[0].T,
        A_mem0[0],
        A_Wq,
        A_Wk,
        A_Wv,
        jnp.transpose(A_Wo, (0, 2, 1)),
        B_w1,
        B_w3,
        B_w2.T,
    )
    return out_t.T[None]
```

```python
import functools
import math

import jax
import jax.numpy as jnp
from jax import lax
import jax.experimental.pallas as pl
import jax.experimental.pallas.tpu as pltpu

F32 = jnp.float32
BF16 = jnp.bfloat16
LANES = 128
LAG = 4
HEAD_GROUP = 2
EDGE_GROUP = 4
N_EARLY = 12
FF_CHUNK = 512
COPY_WINDOW = 3
LN_EPS = 1e-5
MASK_FILL = -1000000000.0
LOG2E = math.log2(math.e)
NT_DIMS = (((1,), (1,)), ((), ()))


def _dot(a, b):
    return jnp.dot(a, b, preferred_element_type=F32)


def _dot_nt(a, b):
    return lax.dot_general(a, b, NT_DIMS, preferred_element_type=F32)


def _as_bf16(words):
    return pltpu.bitcast(words, BF16)


def _block(index, size):
    start = index * size
    return pl.ds(start if isinstance(index, int) else pl.multiple_of(start, size), size)


def _layernorm(x):
    mean = jnp.mean(x, axis=-1, keepdims=True)
    cen = x - mean
    var = jnp.mean(cen * cen, axis=-1, keepdims=True)
    return cen * lax.rsqrt(var + LN_EPS)


def _mask_fill(n_streams, seg, n_mem):
    rows = n_streams * (seg + n_mem)

    def stream_and_pos(i):
        is_mem = i >= n_streams * seg
        j = i - n_streams * seg
        stream = jnp.where(is_mem, j // n_mem, i // seg)
        pos = jnp.where(is_mem, j % n_mem, n_mem + i % seg)
        return stream, pos

    q_stream, q_pos = stream_and_pos(lax.broadcasted_iota(jnp.int32, (rows, rows), 0))
    k_stream, k_pos = stream_and_pos(lax.broadcasted_iota(jnp.int32, (rows, rows), 1))
    visible = (q_pos < n_mem) | (q_pos >= k_pos)
    fill = jnp.where(visible, 0.0, MASK_FILL * LOG2E).astype(F32)
    return jnp.where(q_stream == k_stream, fill, -jnp.inf)


def _kernel(xt_hbm, mem0_ref, wq_hbm, wk_hbm, wv_hbm, wot_hbm, w1_hbm, w3_hbm, w2t_hbm,
            out_hbm,
            xt_buf, stage, early, wqkv, wot, w1, w3, w2t, res, nrm, mem, o_buf, h_buf, ff_main, ff_tail,
            fill1, fill2, sem_x, sem_qkv, sem_o, sem_ff, sem_out,
            *, seg, n_mem, n_heads, head_dim):
    d_model, seq = xt_buf.shape
    d_ff = w1.shape[1]
    d_main = d_model // LANES * LANES
    n_seg = seq // seg
    n_pairs = n_heads // 2
    n_chunks = d_ff // FF_CHUNK
    score_scale = head_dim ** -0.5 * LOG2E
    head_cols = 3 * head_dim

    n_blocks = seq // LANES
    first_early = n_seg - N_EARLY
    late_blocks = first_early * seg // LANES

    def x_copy(block):
        tok = _block(block, LANES)
        return pltpu.make_async_copy(xt_hbm.at[:, tok], xt_buf.at[:, tok], sem_x.at[block])

    def qkv_copy(pair, which):
        src = (wq_hbm, wk_hbm, wv_hbm)[which].bitcast(jnp.uint32)
        return pltpu.make_async_copy(src.at[:, pair, :], stage.at[which, pair],
                                     sem_qkv.at[which, pair])

    def wo_copy(head):
        return pltpu.make_async_copy(wot_hbm.bitcast(jnp.uint32).at[head],
                                     wot.at[:, pl.ds(head * head_dim, head_dim)], sem_o.at[head])

    ff_copies = [pltpu.make_async_copy(src.bitcast(jnp.uint32), dst, sem_ff.at[i])
                 for i, (src, dst) in enumerate(((w1_hbm, w1), (w3_hbm, w3), (w2t_hbm, w2t)))]

    for block in range(late_blocks, n_blocks):
        x_copy(block).start()
    for which in range(3):
        qkv_copy(0, which).start()

    fill1[...] = _mask_fill(1, seg, n_mem)
    fill2[...] = _mask_fill(2, seg, n_mem)
    mem0 = mem0_ref[...].astype(F32)
    mem[0:n_mem, :] = mem0
    mem[n_mem:2 * n_mem, :] = mem0

    ff_main[...] = jnp.zeros(ff_main.shape, F32)
    ff_tail[...] = jnp.zeros(ff_tail.shape, F32)

    for block in range(late_blocks, n_blocks):
        x_copy(block).wait()
    for pair in range(1, COPY_WINDOW):
        for which in range(3):
            qkv_copy(pair, which).start()

    def load_tokens(src_block, dst_block):
        x = xt_buf[:, _block(src_block, LANES)].astype(F32).T
        rows = _block(dst_block, LANES)
        res[rows, :] = x
        nrm[rows, :] = _layernorm(x).astype(BF16)

    for block in range(late_blocks, n_blocks):
        load_tokens(block, block)

    def prepare_pair(pair, carry):
        ahead = pair + COPY_WINDOW
        block = pair - (n_pairs - late_blocks)

        @pl.when(ahead < n_pairs)
        def _():
            for which in range(3):
                qkv_copy(ahead, which).start()

        @pl.when(ahead == n_pairs)
        def _():
            for head in range(n_heads):
                wo_copy(head).start()

        @pl.when(pair < late_blocks)
        def _():
            x_copy(pair).start()

        @pl.when(block >= 0)
        def _():
            x_copy(block).wait()

        for which in range(3):
            qkv_copy(pair, which).wait()
        words = [stage[which, pair] for which in range(3)]
        even = [lax.bitcast_convert_type(w << 16, F32) for w in words]
        odd = [lax.bitcast_convert_type(w & jnp.uint32(0xFFFF0000), F32) for w in words]
        w_pair = jnp.concatenate([w.astype(BF16) for w in even + odd], axis=1)
        cols = _block(pair, 2 * head_cols)
        early[:, cols] = _dot(nrm[first_early * seg:seq, :], w_pair).astype(BF16)
        wqkv[:, cols] = pltpu.bitcast(w_pair, jnp.uint32)
        load_tokens(jnp.where(block < 0, late_blocks, block), jnp.where(block < 0, n_blocks, block))
        return carry

    lax.fori_loop(0, n_pairs, prepare_pair, 0)
    for head in range(n_heads):
        wo_copy(head).wait()
    for copy in ff_copies:
        copy.start()

    def seg_rows(s):
        return _block(s, seg)

    def add_and_normalize(s, delta):
        x = res[seg_rows(s), :] + delta
        normalized = _layernorm(x).astype(BF16)
        res[seg_rows(s), :] = x
        nrm[seg_rows(s), :] = normalized
        return normalized

    def attention_stages(h, fill_ref, group, early_rows=None):
        rows = fill_ref.shape[0]
        n_groups = n_heads // group
        qkv, probs = {}, {}
        for g in range(n_groups + 2):
            if g < n_groups:
                cols = slice(g * group * head_cols, (g + 1) * group * head_cols)
                qkv[g] = _dot(h, _as_bf16(wqkv[:, cols])).astype(BF16)
                if early_rows is not None:
                    qkv[g] = jnp.concatenate([early[early_rows, cols], qkv[g]], axis=0)
            if 0 <= g - 1 < n_groups:
                y = qkv[g - 1]
                probs[g - 1] = []
                for i in range(group):
                    q = y[:, i * head_cols:i * head_cols + head_dim]
                    k = y[:, i * head_cols + head_dim:i * head_cols + 2 * head_dim]
                    fill = fill_ref[...]
                    s = jnp.where(fill == 0.0, _dot_nt(q, k) * score_scale, fill)
                    e = jnp.exp2(s - jnp.max(s, axis=-1, keepdims=True))
                    p = e * (1.0 / jnp.sum(e, axis=-1, keepdims=True))
                    probs[g - 1].append(p.astype(BF16))
            if 0 <= g - 2 < n_groups:
                y = qkv.pop(g - 2)
                for i, p in enumerate(probs.pop(g - 2)):
                    v = y[:, i * head_cols + 2 * head_dim:(i + 1) * head_cols]
                    head = (g - 2) * group + i
                    o_buf[0:rows, head * head_dim:(head + 1) * head_dim] = _dot(p, v).astype(BF16)
            yield g >= n_groups - 1, max(g - 1, 0) * group

    def project_main(act, wt_ref):
        return _dot_nt(act, _as_bf16(wt_ref[0:d_main // 2, :]))

    def project_tail(act, wt_ref):
        return _dot_nt(_as_bf16(wt_ref[d_main // 2:, :]), act)

    def gate_up(hf, c, rows):
        cols = slice(c * FF_CHUNK, (c + 1) * FF_CHUNK)
        gate = _dot(hf, _as_bf16(w1[:, cols]))
        up = _dot(hf, _as_bf16(w3[:, cols]))
        h_buf[rows, cols] = (gate * (1.0 / (1.0 + jnp.exp(-gate))) * up).astype(BF16)

    def ff_input(t):
        sa, sb = ff_blocks(t)
        return jnp.concatenate([nrm[seg_rows(sa), :], nrm[seg_rows(sb), :]], axis=0)

    def ff_finish(segments):
        out = jnp.concatenate([ff_main[...], ff_tail[...].T], axis=1)
        for i, s in enumerate(segments):
            add_and_normalize(s, out[i * seg:(i + 1) * seg, :])

    def ff_blocks(t):
        if isinstance(t, int):
            return t - 1, t - LAG - 1
        return t - 1, jnp.where(t == LAG, t - 2, t - LAG - 1)

    def out_copy(block):
        tok = _block(block, LANES)
        return pltpu.make_async_copy(xt_buf.at[:, tok], out_hbm.at[:, tok], sem_out.at[block])

    def stage_output(block):
        tok = _block(block, LANES)
        xt_buf[:, tok] = res[tok, :].T.astype(BF16)

    def fused_step(t, stages, ff_in, ff_rows, with_tail, lead=0):
        chunks = iter(range(n_chunks))
        for _ in range(lead):
            gate_up(ff_in, next(chunks), ff_rows)
        for draining, _ in stages:
            if draining:
                gate_up(ff_in, next(chunks), ff_rows)
        for c in chunks:
            gate_up(ff_in, c, ff_rows)
        heads = o_buf[...]
        tail = project_tail(heads, wot)
        out = jnp.concatenate([project_main(heads, wot), tail.T], axis=1)
        if with_tail:
            ff_tail[...] = project_tail(h_buf[...], w2t)
        ff_main[ff_rows, :] = project_main(h_buf[ff_rows, :], w2t)
        next_in = jnp.concatenate([add_and_normalize(t, out[0:seg, :]),
                                   add_and_normalize(t - LAG, out[seg:2 * seg, :])], axis=0)
        return out[2 * seg:, :], next_in

    def early_step(t, carry):
        odd = t % 2
        ff_in = ff_input(t)
        pending = ff_blocks(t - 2) + ff_blocks(t - 1)
        ff_finish([jnp.where(odd == 1, n_seg + j, s) for j, s in enumerate(pending)])
        stage_output(t - first_early)
        h = jnp.concatenate([nrm[seg_rows(t - LAG), :], mem[...].astype(BF16)], axis=0)
        stages = attention_stages(h, fill2, HEAD_GROUP, seg_rows(t - first_early))
        ff_rows = _block(odd, 2 * seg)
        mem[...], _ = fused_step(t, stages, ff_in, ff_rows, with_tail=False, lead=1)
        out_copy(t - first_early).start()

        @pl.when(odd == 1)
        def _():
            ff_tail[...] = project_tail(h_buf[...], w2t)

        return carry

    def fused_pair(i, carry):
        t = LAG + 2 * i
        ff_in = ff_input(t)
        pending = ff_blocks(t - 2) + ff_blocks(t - 1)
        ff_finish([jnp.where(i == 0, n_seg + j, s) for j, s in enumerate(pending)])
        memory = mem[...]
        for j in range(2):
            h = jnp.concatenate([nrm[seg_rows(t + j), :], nrm[seg_rows(t + j - LAG), :],
                                 memory.astype(BF16)], axis=0)
            memory, ff_in = fused_step(t + j, attention_stages(h, fill2, HEAD_GROUP), ff_in,
                                       slice(2 * j * seg, 2 * (j + 1) * seg),
                                       with_tail=j == 1, lead=1 - j)
        mem[...] = memory
        return carry

    def edge_step(s=None, layer=None, ff_segments=None):
        ff_rows = slice(0, 2 * seg)
        chunks = iter(range(n_chunks) if ff_segments else ())
        if ff_segments:
            ff_in = jnp.concatenate([nrm[seg_rows(f), :] for f in ff_segments], axis=0)
        if s is not None:
            mem_rows = slice(layer * n_mem, (layer + 1) * n_mem)
            h = jnp.concatenate(
                [nrm[seg_rows(s), :].astype(F32), mem[mem_rows, :]], axis=0).astype(BF16)
            parts, projected = [], 0

            def project(stop):
                cols = slice(projected * head_dim, stop * head_dim)
                parts.append(_dot_nt(o_buf[0:seg + n_mem, cols], _as_bf16(wot[:, cols])))
                return stop

            for draining, finished in attention_stages(h, fill1, EDGE_GROUP):
                if draining and ff_segments:
                    gate_up(ff_in, next(chunks), ff_rows)
                elif draining and finished < n_heads:
                    projected = project(min(finished, projected + 3 * n_heads // 8))
        for c in chunks:
            gate_up(ff_in, c, ff_rows)
        if s is not None:
            project(n_heads)
            out = functools.reduce(jnp.add, parts)
        if ff_segments:
            ff_out = _dot_nt(h_buf[ff_rows, :], _as_bf16(w2t[...]))
        if s is not None:
            mem[mem_rows, :] = out[seg:, :]
            add_and_normalize(s, out[0:seg, :])
        for i, f in enumerate(ff_segments or ()):
            add_and_normalize(f, ff_out[i * seg:(i + 1) * seg, :])

    def head_step(s, carry):
        edge_step(s, 0)
        return carry

    finished_blocks = (n_seg - LAG - 1) * seg // LANES
    tail_blocks = (finished_blocks - N_EARLY) // (LAG // 2)
    assert tail_blocks >= 0

    def tail_pair(i, carry):
        s = n_seg - LAG + 2 * i
        blocks = [N_EARLY + tail_blocks * i + j for j in range(tail_blocks)]
        for block in blocks:
            stage_output(block)
        edge_step(s, 1, (jnp.where(i == 0, n_seg - 1, s - 2), s - 1))
        for block in blocks:
            out_copy(block).start()
        edge_step(s + 1, 1)
        return carry

    lax.fori_loop(0, LAG, head_step, 0)
    for copy in ff_copies:
        copy.wait()
    edge_step(ff_segments=(0, 1))
    lax.fori_loop(0, (first_early - LAG) // 2, fused_pair, 0)
    lax.fori_loop(first_early, n_seg, early_step, 0)
    ff_finish(ff_blocks(n_seg - 2) + ff_blocks(n_seg - 1))
    lax.fori_loop(0, LAG // 2, tail_pair, 0)
    edge_step(ff_segments=(n_seg - 2, n_seg - 1))
    for block in range(N_EARLY + tail_blocks * (LAG // 2), n_blocks):
        stage_output(block)
        out_copy(block).start()
    for block in range(n_blocks):
        out_copy(block).wait()


@functools.partial(jax.jit, static_argnames=("A_seg_len",))
def pallas_interleave_layers__memory_aug_recurrent_mem_tr__glu_gated_swiglu__prompt_kernel(
    A_x: jax.Array,
    A_mem0: jax.Array,
    A_Wq: jax.Array,
    A_Wk: jax.Array,
    A_Wv: jax.Array,
    A_Wo: jax.Array,
    A_seg_len: int,
    B_x: jax.Array,
    B_w1: jax.Array,
    B_w3: jax.Array,
    B_w2: jax.Array,
):
    del B_x
    batch, seq, d_model = A_x.shape
    n_mem = A_mem0.shape[1]
    _, n_heads, head_dim = A_Wq.shape
    d_ff = B_w1.shape[1]
    seg = int(A_seg_len)
    assert batch == 1 and seq % LANES == 0 and seq % seg == 0 and head_dim == LANES
    assert d_ff % FF_CHUNK == 0 and n_heads % HEAD_GROUP == 0 and N_EARLY % 2 == 0 and LAG == 4
    rows = 2 * (seg + n_mem)

    any_spec = pl.BlockSpec(memory_space=pl.ANY)
    out_t = pl.pallas_call(
        functools.partial(_kernel, seg=seg, n_mem=n_mem, n_heads=n_heads, head_dim=head_dim),
        out_shape=jax.ShapeDtypeStruct((d_model, seq), A_x.dtype),
        in_specs=[any_spec, pl.BlockSpec(memory_space=pltpu.VMEM)] + [any_spec] * 7,
        out_specs=any_spec,
        scratch_shapes=[
            pltpu.VMEM((d_model, seq), BF16),
            pltpu.VMEM((3, n_heads // 2, d_model, head_dim), jnp.uint32),
            pltpu.VMEM((N_EARLY * seg, 3 * n_heads * head_dim), BF16),
            pltpu.VMEM((d_model // 2, 3 * n_heads * head_dim), jnp.uint32),
            pltpu.VMEM((d_model // 2, n_heads * head_dim), jnp.uint32),
            pltpu.VMEM((d_model // 2, d_ff), jnp.uint32),
            pltpu.VMEM((d_model // 2, d_ff), jnp.uint32),
            pltpu.VMEM((d_model // 2, d_ff), jnp.uint32),
            pltpu.VMEM((seq + 4 * seg, d_model), F32),
            pltpu.VMEM((seq + 4 * seg, d_model), BF16),
            pltpu.VMEM((2 * n_mem, d_model), F32),
            pltpu.VMEM((rows, n_heads * head_dim), BF16),
            pltpu.VMEM((4 * seg, d_ff), BF16),
            pltpu.VMEM((4 * seg, d_model // LANES * LANES), F32),
            pltpu.VMEM((d_model % LANES, 4 * seg), F32),
            pltpu.VMEM((rows // 2, rows // 2), F32),
            pltpu.VMEM((rows, rows), F32),
            pltpu.SemaphoreType.DMA((seq // LANES,)),
            pltpu.SemaphoreType.DMA((3, n_heads // 2)),
            pltpu.SemaphoreType.DMA((n_heads,)),
            pltpu.SemaphoreType.DMA((3,)),
            pltpu.SemaphoreType.DMA((seq // LANES,)),
        ],
        compiler_params=pltpu.CompilerParams(vmem_limit_bytes=100 * 1024 * 1024),
    )(
        A_x[0].T,
        A_mem0[0],
        A_Wq,
        A_Wk,
        A_Wv,
        jnp.transpose(A_Wo, (0, 2, 1)),
        B_w1,
        B_w3,
        B_w2.T,
    )
    return out_t.T[None]
```

```python
import functools
import math

import jax
import jax.numpy as jnp
from jax import lax
import jax.experimental.pallas as pl
import jax.experimental.pallas.tpu as pltpu

F32 = jnp.float32
BF16 = jnp.bfloat16
LANES = 128
LAG = 4
HEAD_GROUP = 2
EDGE_GROUP = 4
N_EARLY = 12
FF_CHUNK = 512
COPY_WINDOW = 3
LN_EPS = 1e-5
MASK_FILL = -1000000000.0
LOG2E = math.log2(math.e)
NT_DIMS = (((1,), (1,)), ((), ()))


def _dot(a, b):
    return jnp.dot(a, b, preferred_element_type=F32)


def _dot_nt(a, b):
    return lax.dot_general(a, b, NT_DIMS, preferred_element_type=F32)


def _as_bf16(words):
    return pltpu.bitcast(words, BF16)


def _block(index, size):
    start = index * size
    return pl.ds(start if isinstance(index, int) else pl.multiple_of(start, size), size)


def _layernorm(x):
    mean = jnp.mean(x, axis=-1, keepdims=True)
    cen = x - mean
    var = jnp.mean(cen * cen, axis=-1, keepdims=True)
    return cen * lax.rsqrt(var + LN_EPS)


def _mask_fill(n_streams, seg, n_mem):
    rows = n_streams * (seg + n_mem)

    def stream_and_pos(i):
        is_mem = i >= n_streams * seg
        j = i - n_streams * seg
        stream = jnp.where(is_mem, j // n_mem, i // seg)
        pos = jnp.where(is_mem, j % n_mem, n_mem + i % seg)
        return stream, pos

    q_stream, q_pos = stream_and_pos(lax.broadcasted_iota(jnp.int32, (rows, rows), 0))
    k_stream, k_pos = stream_and_pos(lax.broadcasted_iota(jnp.int32, (rows, rows), 1))
    visible = (q_pos < n_mem) | (q_pos >= k_pos)
    fill = jnp.where(visible, 0.0, MASK_FILL * LOG2E).astype(F32)
    return jnp.where(q_stream == k_stream, fill, -jnp.inf)


def _kernel(xt_hbm, mem0_ref, wq_hbm, wk_hbm, wv_hbm, wot_hbm, w1_hbm, w3_hbm, w2t_hbm,
            out_hbm,
            xt_buf, stage, early, rider_in, rider, wqkv, wot, w1, w3, w2t, res, nrm, mem, o_buf, h_buf, ff_main, ff_tail,
            fill1, fill2, sem_x, sem_qkv, sem_o, sem_ff, sem_out,
            *, seg, n_mem, n_heads, head_dim):
    d_model, seq = xt_buf.shape
    d_ff = w1.shape[1]
    d_main = d_model // LANES * LANES
    n_seg = seq // seg
    n_pairs = n_heads // 2
    n_chunks = d_ff // FF_CHUNK
    score_scale = head_dim ** -0.5 * LOG2E
    head_cols = 3 * head_dim

    n_blocks = seq // LANES
    first_early = n_seg - N_EARLY
    late_blocks = first_early * seg // LANES

    def x_copy(block):
        tok = _block(block, LANES)
        return pltpu.make_async_copy(xt_hbm.at[:, tok], xt_buf.at[:, tok], sem_x.at[block])

    def qkv_copy(pair, which):
        src = (wq_hbm, wk_hbm, wv_hbm)[which].bitcast(jnp.uint32)
        return pltpu.make_async_copy(src.at[:, pair, :], stage.at[which, pair],
                                     sem_qkv.at[which, pair])

    def wo_copy(head):
        return pltpu.make_async_copy(wot_hbm.bitcast(jnp.uint32).at[head],
                                     wot.at[:, pl.ds(head * head_dim, head_dim)], sem_o.at[head])

    ff_copies = [pltpu.make_async_copy(src.bitcast(jnp.uint32), dst, sem_ff.at[i])
                 for i, (src, dst) in enumerate(((w1_hbm, w1), (w3_hbm, w3), (w2t_hbm, w2t)))]

    for block in range(late_blocks, n_blocks):
        x_copy(block).start()
    for which in range(3):
        qkv_copy(0, which).start()

    fill1[...] = _mask_fill(1, seg, n_mem)
    fill2[...] = _mask_fill(2, seg, n_mem)
    mem0 = mem0_ref[...].astype(F32)
    mem[0:n_mem, :] = mem0
    mem[n_mem:2 * n_mem, :] = mem0

    ff_main[...] = jnp.zeros(ff_main.shape, F32)
    ff_tail[...] = jnp.zeros(ff_tail.shape, F32)

    for block in range(late_blocks, n_blocks):
        x_copy(block).wait()
    for pair in range(1, COPY_WINDOW):
        for which in range(3):
            qkv_copy(pair, which).start()

    def load_tokens(src_block, dst_block):
        x = xt_buf[:, _block(src_block, LANES)].astype(F32).T
        rows = _block(dst_block, LANES)
        res[rows, :] = x
        nrm[rows, :] = _layernorm(x).astype(BF16)

    for block in range(late_blocks, n_blocks):
        load_tokens(block, block)

    def prepare_pair(pair, carry):
        ahead = pair + COPY_WINDOW
        block = pair - (n_pairs - late_blocks)

        @pl.when(ahead < n_pairs)
        def _():
            for which in range(3):
                qkv_copy(ahead, which).start()

        @pl.when(ahead == n_pairs)
        def _():
            for head in range(n_heads):
                wo_copy(head).start()

        @pl.when(pair < late_blocks)
        def _():
            x_copy(pair).start()

        @pl.when(block >= 0)
        def _():
            x_copy(block).wait()

        for which in range(3):
            qkv_copy(pair, which).wait()
        words = [stage[which, pair] for which in range(3)]
        even = [lax.bitcast_convert_type(w << 16, F32) for w in words]
        odd = [lax.bitcast_convert_type(w & jnp.uint32(0xFFFF0000), F32) for w in words]
        w_pair = jnp.concatenate([w.astype(BF16) for w in even + odd], axis=1)
        cols = _block(pair, 2 * head_cols)
        early[0:(N_EARLY - 1) * seg, cols] = _dot(
            nrm[first_early * seg:seq - seg, :], w_pair).astype(BF16)
        wqkv[:, cols] = pltpu.bitcast(w_pair, jnp.uint32)
        load_tokens(jnp.where(block < 0, late_blocks, block), jnp.where(block < 0, n_blocks, block))
        return carry

    lax.fori_loop(0, n_pairs, prepare_pair, 0)
    for head in range(n_heads):
        wo_copy(head).wait()
    for copy in ff_copies:
        copy.start()

    def seg_rows(s):
        return _block(s, seg)

    def add_and_normalize(s, delta):
        x = res[seg_rows(s), :] + delta
        normalized = _layernorm(x).astype(BF16)
        res[seg_rows(s), :] = x
        nrm[seg_rows(s), :] = normalized
        return normalized

    def attention_stages(h, fill_ref, group, early_rows=None, rider_rows=None):
        rows = fill_ref.shape[0]
        n_groups = n_heads // group
        qkv, probs = {}, {}
        for g in range(n_groups + 2):
            if g < n_groups:
                cols = slice(g * group * head_cols, (g + 1) * group * head_cols)
                y = _dot(h, _as_bf16(wqkv[:, cols]))
                if rider_rows is not None:
                    rider[rider_rows, cols] = y[rows:, :]
                    y = y[0:rows, :]
                qkv[g] = y.astype(BF16)
                if early_rows is not None:
                    qkv[g] = jnp.concatenate([early[early_rows, cols], qkv[g]], axis=0)
            if 0 <= g - 1 < n_groups:
                y = qkv[g - 1]
                probs[g - 1] = []
                for i in range(group):
                    q = y[:, i * head_cols:i * head_cols + head_dim]
                    k = y[:, i * head_cols + head_dim:i * head_cols + 2 * head_dim]
                    fill = fill_ref[...]
                    s = jnp.where(fill == 0.0, _dot_nt(q, k) * score_scale, fill)
                    e = jnp.exp2(s - jnp.max(s, axis=-1, keepdims=True))
                    p = e * (1.0 / jnp.sum(e, axis=-1, keepdims=True))
                    probs[g - 1].append(p.astype(BF16))
            if 0 <= g - 2 < n_groups:
                y = qkv.pop(g - 2)
                for i, p in enumerate(probs.pop(g - 2)):
                    v = y[:, i * head_cols + 2 * head_dim:(i + 1) * head_cols]
                    head = (g - 2) * group + i
                    o_buf[0:rows, head * head_dim:(head + 1) * head_dim] = _dot(p, v).astype(BF16)
            yield g >= n_groups - 1, max(g - 1, 0) * group

    def project_main(act, wt_ref):
        return _dot_nt(act, _as_bf16(wt_ref[0:d_main // 2, :]))

    def project_tail(act, wt_ref):
        return _dot_nt(_as_bf16(wt_ref[d_main // 2:, :]), act)

    def gate_up(hf, c, rows):
        cols = slice(c * FF_CHUNK, (c + 1) * FF_CHUNK)
        gate = _dot(hf, _as_bf16(w1[:, cols]))
        up = _dot(hf, _as_bf16(w3[:, cols]))
        h_buf[rows, cols] = (gate * (1.0 / (1.0 + jnp.exp(-gate))) * up).astype(BF16)

    def ff_input(t):
        sa, sb = ff_blocks(t)
        return jnp.concatenate([nrm[seg_rows(sa), :], nrm[seg_rows(sb), :]], axis=0)

    def ff_finish(segments):
        out = jnp.concatenate([ff_main[...], ff_tail[...].T], axis=1)
        for i, s in enumerate(segments):
            add_and_normalize(s, out[i * seg:(i + 1) * seg, :])

    def ff_blocks(t):
        if isinstance(t, int):
            return t - 1, t - LAG - 1
        return t - 1, jnp.where(t == LAG, t - 2, t - LAG - 1)

    def out_copy(block):
        tok = _block(block, LANES)
        return pltpu.make_async_copy(xt_buf.at[:, tok], out_hbm.at[:, tok], sem_out.at[block])

    def stage_output(block):
        tok = _block(block, LANES)
        xt_buf[:, tok] = res[tok, :].T.astype(BF16)

    def fused_step(t, stages, ff_in, ff_rows, with_tail, lead=0):
        chunks = iter(range(n_chunks))
        for _ in range(lead):
            gate_up(ff_in, next(chunks), ff_rows)
        for draining, _ in stages:
            if draining:
                gate_up(ff_in, next(chunks), ff_rows)
        for c in chunks:
            gate_up(ff_in, c, ff_rows)
        heads = o_buf[...]
        tail = project_tail(heads, wot)
        out = jnp.concatenate([project_main(heads, wot), tail.T], axis=1)
        if with_tail:
            ff_tail[...] = project_tail(h_buf[...], w2t)
        ff_main[ff_rows, :] = project_main(h_buf[ff_rows, :], w2t)
        next_in = jnp.concatenate([add_and_normalize(t, out[0:seg, :]),
                                   add_and_normalize(t - LAG, out[seg:2 * seg, :])], axis=0)
        return out[2 * seg:, :], next_in

    def early_step(t, carry):
        odd = t % 2
        ff_in = ff_input(t)
        pending = ff_blocks(t - 2) + ff_blocks(t - 1)
        ff_finish([jnp.where(odd == 1, n_seg + j, s) for j, s in enumerate(pending)])
        stage_output(t - first_early)
        h = jnp.concatenate([nrm[seg_rows(t - LAG), :], mem[...].astype(BF16)], axis=0)
        stages = attention_stages(h, fill2, HEAD_GROUP, seg_rows(t - first_early))
        ff_rows = _block(odd, 2 * seg)
        mem[...], _ = fused_step(t, stages, ff_in, ff_rows, with_tail=False, lead=1)
        out_copy(t - first_early).start()

        @pl.when(odd == 1)
        def _():
            ff_tail[...] = project_tail(h_buf[...], w2t)

        return carry

    def fused_pair(i, carry):
        t = LAG + 2 * i
        ff_in = ff_input(t)
        pending = ff_blocks(t - 2) + ff_blocks(t - 1)
        ff_finish([jnp.where(i == 0, n_seg + j, s) for j, s in enumerate(pending)])
        memory = mem[...]
        for j in range(2):
            h = jnp.concatenate([nrm[seg_rows(t + j), :], nrm[seg_rows(t + j - LAG), :],
                                 memory.astype(BF16)], axis=0)
            memory, ff_in = fused_step(t + j, attention_stages(h, fill2, HEAD_GROUP), ff_in,
                                       slice(2 * j * seg, 2 * (j + 1) * seg),
                                       with_tail=j == 1, lead=1 - j)
        mem[...] = memory
        return carry

    def edge_step(s=None, layer=None, ff_segments=None):
        ff_rows = slice(0, 2 * seg)
        chunks = iter(range(n_chunks) if ff_segments else ())
        if ff_segments:
            ff_in = jnp.concatenate([nrm[seg_rows(f), :] for f in ff_segments], axis=0)
        if s is not None:
            mem_rows = slice(layer * n_mem, (layer + 1) * n_mem)
            h = [nrm[seg_rows(s), :].astype(F32), mem[mem_rows, :]]
            rider_rows = None
            if layer == 0:
                rider_rows = _block(s, n_mem)
                h.append(rider_in[rider_rows, :])
            h = jnp.concatenate(h, axis=0).astype(BF16)
            parts, projected = [], 0

            def project(stop):
                cols = slice(projected * head_dim, stop * head_dim)
                parts.append(_dot_nt(o_buf[0:seg + n_mem, cols], _as_bf16(wot[:, cols])))
                return stop

            for draining, finished in attention_stages(h, fill1, EDGE_GROUP,
                                                       rider_rows=rider_rows):
                if draining and ff_segments:
                    gate_up(ff_in, next(chunks), ff_rows)
                elif draining and finished < n_heads:
                    projected = project(min(finished, projected + 3 * n_heads // 8))
        for c in chunks:
            gate_up(ff_in, c, ff_rows)
        if s is not None:
            project(n_heads)
            out = functools.reduce(jnp.add, parts)
        if ff_segments:
            ff_out = _dot_nt(h_buf[ff_rows, :], _as_bf16(w2t[...]))
        if s is not None:
            mem[mem_rows, :] = out[seg:, :]
            add_and_normalize(s, out[0:seg, :])
        for i, f in enumerate(ff_segments or ()):
            add_and_normalize(f, ff_out[i * seg:(i + 1) * seg, :])

    def head_step(s, carry):
        edge_step(s, 0)
        return carry

    finished_blocks = (n_seg - LAG - 1) * seg // LANES
    tail_blocks = (finished_blocks - N_EARLY) // (LAG // 2)
    assert tail_blocks >= 0

    def tail_pair(i, carry):
        s = n_seg - LAG + 2 * i
        blocks = [N_EARLY + tail_blocks * i + j for j in range(tail_blocks)]
        for block in blocks:
            stage_output(block)
        edge_step(s, 1, (jnp.where(i == 0, n_seg - 1, s - 2), s - 1))
        for block in blocks:
            out_copy(block).start()
        edge_step(s + 1, 1)
        return carry

    rider_in[...] = nrm[seq - seg:seq, :].astype(F32)
    lax.fori_loop(0, LAG, head_step, 0)
    for copy in ff_copies:
        copy.wait()
    early[(N_EARLY - 1) * seg:, :] = rider[...].astype(BF16)
    edge_step(ff_segments=(0, 1))
    lax.fori_loop(0, (first_early - LAG) // 2, fused_pair, 0)
    lax.fori_loop(first_early, n_seg, early_step, 0)
    ff_finish(ff_blocks(n_seg - 2) + ff_blocks(n_seg - 1))
    lax.fori_loop(0, LAG // 2, tail_pair, 0)
    edge_step(ff_segments=(n_seg - 2, n_seg - 1))
    for block in range(N_EARLY + tail_blocks * (LAG // 2), n_blocks):
        stage_output(block)
        out_copy(block).start()
    for block in range(n_blocks):
        out_copy(block).wait()


@functools.partial(jax.jit, static_argnames=("A_seg_len",))
def pallas_interleave_layers__memory_aug_recurrent_mem_tr__glu_gated_swiglu__prompt_kernel(
    A_x: jax.Array,
    A_mem0: jax.Array,
    A_Wq: jax.Array,
    A_Wk: jax.Array,
    A_Wv: jax.Array,
    A_Wo: jax.Array,
    A_seg_len: int,
    B_x: jax.Array,
    B_w1: jax.Array,
    B_w3: jax.Array,
    B_w2: jax.Array,
):
    del B_x
    batch, seq, d_model = A_x.shape
    n_mem = A_mem0.shape[1]
    _, n_heads, head_dim = A_Wq.shape
    d_ff = B_w1.shape[1]
    seg = int(A_seg_len)
    assert batch == 1 and seq % LANES == 0 and seq % seg == 0 and head_dim == LANES
    assert d_ff % FF_CHUNK == 0 and n_heads % HEAD_GROUP == 0 and N_EARLY % 2 == 0 and LAG == 4 and LAG * n_mem == seg
    rows = 2 * (seg + n_mem)

    any_spec = pl.BlockSpec(memory_space=pl.ANY)
    out_t = pl.pallas_call(
        functools.partial(_kernel, seg=seg, n_mem=n_mem, n_heads=n_heads, head_dim=head_dim),
        out_shape=jax.ShapeDtypeStruct((d_model, seq), A_x.dtype),
        in_specs=[any_spec, pl.BlockSpec(memory_space=pltpu.VMEM)] + [any_spec] * 7,
        out_specs=any_spec,
        scratch_shapes=[
            pltpu.VMEM((d_model, seq), BF16),
            pltpu.VMEM((3, n_heads // 2, d_model, head_dim), jnp.uint32),
            pltpu.VMEM((N_EARLY * seg, 3 * n_heads * head_dim), BF16),
            pltpu.VMEM((seg, d_model), F32),
            pltpu.VMEM((seg, 3 * n_heads * head_dim), F32),
            pltpu.VMEM((d_model // 2, 3 * n_heads * head_dim), jnp.uint32),
            pltpu.VMEM((d_model // 2, n_heads * head_dim), jnp.uint32),
            pltpu.VMEM((d_model // 2, d_ff), jnp.uint32),
            pltpu.VMEM((d_model // 2, d_ff), jnp.uint32),
            pltpu.VMEM((d_model // 2, d_ff), jnp.uint32),
            pltpu.VMEM((seq + 4 * seg, d_model), F32),
            pltpu.VMEM((seq + 4 * seg, d_model), BF16),
            pltpu.VMEM((2 * n_mem, d_model), F32),
            pltpu.VMEM((rows, n_heads * head_dim), BF16),
            pltpu.VMEM((4 * seg, d_ff), BF16),
            pltpu.VMEM((4 * seg, d_model // LANES * LANES), F32),
            pltpu.VMEM((d_model % LANES, 4 * seg), F32),
            pltpu.VMEM((rows // 2, rows // 2), F32),
            pltpu.VMEM((rows, rows), F32),
            pltpu.SemaphoreType.DMA((seq // LANES,)),
            pltpu.SemaphoreType.DMA((3, n_heads // 2)),
            pltpu.SemaphoreType.DMA((n_heads,)),
            pltpu.SemaphoreType.DMA((3,)),
            pltpu.SemaphoreType.DMA((seq // LANES,)),
        ],
        compiler_params=pltpu.CompilerParams(vmem_limit_bytes=100 * 1024 * 1024),
    )(
        A_x[0].T,
        A_mem0[0],
        A_Wq,
        A_Wk,
        A_Wv,
        jnp.transpose(A_Wo, (0, 2, 1)),
        B_w1,
        B_w3,
        B_w2.T,
    )
    return out_t.T[None]
```

```python
import functools
import math

import jax
import jax.numpy as jnp
from jax import lax
import jax.experimental.pallas as pl
import jax.experimental.pallas.tpu as pltpu

F32 = jnp.float32
BF16 = jnp.bfloat16
LANES = 128
LAG = 4
HEAD_GROUP = 2
EDGE_GROUP = 4
N_EARLY = 12
FF_CHUNK = 512
COPY_WINDOW = 3
LN_EPS = 1e-5
MASK_FILL = -1000000000.0
LOG2E = math.log2(math.e)
NT_DIMS = (((1,), (1,)), ((), ()))


def _dot(a, b):
    return jnp.dot(a, b, preferred_element_type=F32)


def _dot_nt(a, b):
    return lax.dot_general(a, b, NT_DIMS, preferred_element_type=F32)


def _as_bf16(words):
    return pltpu.bitcast(words, BF16)


def _block(index, size):
    start = index * size
    return pl.ds(start if isinstance(index, int) else pl.multiple_of(start, size), size)


def _layernorm(x):
    mean = jnp.mean(x, axis=-1, keepdims=True)
    cen = x - mean
    var = jnp.mean(cen * cen, axis=-1, keepdims=True)
    return cen * lax.rsqrt(var + LN_EPS)


def _mask_fill(n_streams, seg, n_mem):
    rows = n_streams * (seg + n_mem)

    def stream_and_pos(i):
        is_mem = i >= n_streams * seg
        j = i - n_streams * seg
        stream = jnp.where(is_mem, j // n_mem, i // seg)
        pos = jnp.where(is_mem, j % n_mem, n_mem + i % seg)
        return stream, pos

    q_stream, q_pos = stream_and_pos(lax.broadcasted_iota(jnp.int32, (rows, rows), 0))
    k_stream, k_pos = stream_and_pos(lax.broadcasted_iota(jnp.int32, (rows, rows), 1))
    visible = (q_pos < n_mem) | (q_pos >= k_pos)
    fill = jnp.where(visible, 0.0, MASK_FILL * LOG2E).astype(F32)
    return jnp.where(q_stream == k_stream, fill, -jnp.inf)


def _kernel(xt_hbm, mem0_ref, wq_hbm, wk_hbm, wv_hbm, wot_hbm, w1_hbm, w3_hbm, w2t_hbm,
            out_hbm,
            xt_buf, stage, early, rider_in, rider, wqkv, wot, w1, w3, w2t, res, nrm, mem, o_buf, h_buf, ff_main, ff_tail,
            fill1, fill2, sem_x, sem_qkv, sem_o, sem_ff, sem_out,
            *, seg, n_mem, n_heads, head_dim):
    d_model, seq = xt_buf.shape
    d_ff = w1.shape[1]
    d_main = d_model // LANES * LANES
    n_seg = seq // seg
    n_pairs = n_heads // 2
    n_chunks = d_ff // FF_CHUNK
    score_scale = head_dim ** -0.5 * LOG2E
    head_cols = 3 * head_dim

    n_blocks = seq // LANES
    first_early = n_seg - N_EARLY
    late_blocks = first_early * seg // LANES

    def x_copy(block):
        tok = _block(block, LANES)
        return pltpu.make_async_copy(xt_hbm.at[:, tok], xt_buf.at[:, tok], sem_x.at[block])

    def qkv_copy(pair, which):
        src = (wq_hbm, wk_hbm, wv_hbm)[which].bitcast(jnp.uint32)
        return pltpu.make_async_copy(src.at[:, pair, :], stage.at[which, pair],
                                     sem_qkv.at[which, pair])

    def wo_copy(head):
        return pltpu.make_async_copy(wot_hbm.bitcast(jnp.uint32).at[head],
                                     wot.at[:, pl.ds(head * head_dim, head_dim)], sem_o.at[head])

    ff_copies = [pltpu.make_async_copy(src.bitcast(jnp.uint32), dst, sem_ff.at[i])
                 for i, (src, dst) in enumerate(((w1_hbm, w1), (w3_hbm, w3), (w2t_hbm, w2t)))]

    for block in range(late_blocks, n_blocks):
        x_copy(block).start()
    for which in range(3):
        qkv_copy(0, which).start()

    fill1[...] = _mask_fill(1, seg, n_mem)
    fill2[...] = _mask_fill(2, seg, n_mem)
    mem0 = mem0_ref[...].astype(F32)
    mem[0:n_mem, :] = mem0
    mem[n_mem:2 * n_mem, :] = mem0

    ff_main[...] = jnp.zeros(ff_main.shape, F32)
    ff_tail[...] = jnp.zeros(ff_tail.shape, F32)

    for block in range(late_blocks, n_blocks):
        x_copy(block).wait()
    for pair in range(1, COPY_WINDOW):
        for which in range(3):
            qkv_copy(pair, which).start()

    def load_tokens(src_block, dst_block):
        x = xt_buf[:, _block(src_block, LANES)].astype(F32).T
        rows = _block(dst_block, LANES)
        res[rows, :] = x
        nrm[rows, :] = _layernorm(x).astype(BF16)

    for block in range(late_blocks, n_blocks):
        load_tokens(block, block)

    def prepare_pair(pair, carry):
        ahead = pair + COPY_WINDOW
        block = pair - (n_pairs - late_blocks)

        @pl.when(ahead < n_pairs)
        def _():
            for which in range(3):
                qkv_copy(ahead, which).start()

        @pl.when(ahead == n_pairs)
        def _():
            for head in range(n_heads):
                wo_copy(head).start()

        @pl.when(pair < late_blocks)
        def _():
            x_copy(pair).start()

        @pl.when(block >= 0)
        def _():
            x_copy(block).wait()

        for which in range(3):
            qkv_copy(pair, which).wait()
        words = [stage[which, pair] for which in range(3)]
        even = [lax.bitcast_convert_type(w << 16, F32) for w in words]
        odd = [lax.bitcast_convert_type(w & jnp.uint32(0xFFFF0000), F32) for w in words]
        w_pair = jnp.concatenate([w.astype(BF16) for w in even + odd], axis=1)
        cols = _block(pair, 2 * head_cols)
        early[0:(N_EARLY - 1) * seg, cols] = _dot(
            nrm[first_early * seg:seq - seg, :], w_pair).astype(BF16)
        wqkv[:, cols] = pltpu.bitcast(w_pair, jnp.uint32)
        load_tokens(jnp.where(block < 0, late_blocks, block), jnp.where(block < 0, n_blocks, block))
        return carry

    lax.fori_loop(0, n_pairs, prepare_pair, 0)
    for head in range(n_heads):
        wo_copy(head).wait()
    for copy in ff_copies:
        copy.start()

    def seg_rows(s):
        return _block(s, seg)

    def add_and_normalize(s, delta):
        x = res[seg_rows(s), :] + delta
        normalized = _layernorm(x).astype(BF16)
        res[seg_rows(s), :] = x
        nrm[seg_rows(s), :] = normalized
        return normalized

    def attention_stages(h, fill_ref, group, arrange=lambda y, cols: y.astype(BF16)):
        rows = fill_ref.shape[0]
        n_groups = n_heads // group
        qkv, probs = {}, {}
        for g in range(n_groups + 2):
            if g < n_groups:
                cols = slice(g * group * head_cols, (g + 1) * group * head_cols)
                qkv[g] = arrange(_dot(h, _as_bf16(wqkv[:, cols])), cols)
            if 0 <= g - 1 < n_groups:
                y = qkv[g - 1]
                probs[g - 1] = []
                for i in range(group):
                    q = y[:, i * head_cols:i * head_cols + head_dim]
                    k = y[:, i * head_cols + head_dim:i * head_cols + 2 * head_dim]
                    fill = fill_ref[...]
                    s = jnp.where(fill == 0.0, _dot_nt(q, k) * score_scale, fill)
                    e = jnp.exp2(s - jnp.max(s, axis=-1, keepdims=True))
                    p = e * (1.0 / jnp.sum(e, axis=-1, keepdims=True))
                    probs[g - 1].append(p.astype(BF16))
            if 0 <= g - 2 < n_groups:
                y = qkv.pop(g - 2)
                for i, p in enumerate(probs.pop(g - 2)):
                    v = y[:, i * head_cols + 2 * head_dim:(i + 1) * head_cols]
                    head = (g - 2) * group + i
                    o_buf[0:rows, head * head_dim:(head + 1) * head_dim] = _dot(p, v).astype(BF16)
            yield g >= n_groups - 1, max(g - 1, 0) * group

    def project_main(act, wt_ref):
        return _dot_nt(act, _as_bf16(wt_ref[0:d_main // 2, :]))

    def project_tail(act, wt_ref):
        return _dot_nt(_as_bf16(wt_ref[d_main // 2:, :]), act)

    def gate_up(hf, c, rows):
        cols = slice(c * FF_CHUNK, (c + 1) * FF_CHUNK)
        gate = _dot(hf, _as_bf16(w1[:, cols]))
        up = _dot(hf, _as_bf16(w3[:, cols]))
        h_buf[rows, cols] = (gate * (1.0 / (1.0 + jnp.exp(-gate))) * up).astype(BF16)

    def ff_input(t):
        sa, sb = ff_blocks(t)
        return jnp.concatenate([nrm[seg_rows(sa), :], nrm[seg_rows(sb), :]], axis=0)

    def ff_finish(segments):
        out = jnp.concatenate([ff_main[...], ff_tail[...].T], axis=1)
        for i, s in enumerate(segments):
            add_and_normalize(s, out[i * seg:(i + 1) * seg, :])

    def ff_blocks(t):
        if isinstance(t, int):
            return t - 1, t - LAG - 1
        return t - 1, jnp.where(t == LAG, t - 2, t - LAG - 1)

    def out_copy(block):
        tok = _block(block, LANES)
        return pltpu.make_async_copy(xt_buf.at[:, tok], out_hbm.at[:, tok], sem_out.at[block])

    def stage_output(block):
        tok = _block(block, LANES)
        xt_buf[:, tok] = res[tok, :].T.astype(BF16)

    def fused_step(t, stages, ff_in, ff_rows, with_tail, lead=0):
        chunks = iter(range(n_chunks))
        for _ in range(lead):
            gate_up(ff_in, next(chunks), ff_rows)
        for draining, _ in stages:
            if draining:
                gate_up(ff_in, next(chunks), ff_rows)
        for c in chunks:
            gate_up(ff_in, c, ff_rows)
        heads = o_buf[...]
        tail = project_tail(heads, wot)
        out = jnp.concatenate([project_main(heads, wot), tail.T], axis=1)
        if with_tail:
            ff_tail[...] = project_tail(h_buf[...], w2t)
        ff_main[ff_rows, :] = project_main(h_buf[ff_rows, :], w2t)
        next_in = jnp.concatenate([add_and_normalize(t, out[0:seg, :]),
                                   add_and_normalize(t - LAG, out[seg:2 * seg, :])], axis=0)
        return out[2 * seg:, :], next_in

    def early_step(t, carry):
        odd = t % 2
        ff_in = ff_input(t)
        pending = ff_blocks(t - 2) + ff_blocks(t - 1)
        ff_finish([jnp.where(odd == 1, n_seg + j, s) for j, s in enumerate(pending)])
        stage_output(t - first_early)
        h = jnp.concatenate([nrm[seg_rows(t - LAG), :], mem[...].astype(BF16)], axis=0)

        def prepend_early(y, cols):
            return jnp.concatenate([early[seg_rows(t - first_early), cols], y.astype(BF16)], axis=0)

        stages = attention_stages(h, fill2, HEAD_GROUP, prepend_early)
        ff_rows = _block(odd, 2 * seg)
        mem[...], _ = fused_step(t, stages, ff_in, ff_rows, with_tail=False, lead=1)
        out_copy(t - first_early).start()

        @pl.when(odd == 1)
        def _():
            ff_tail[...] = project_tail(h_buf[...], w2t)

        return carry

    def fused_pair(i, carry):
        t = LAG + 2 * i
        ff_in = ff_input(t)
        pending = ff_blocks(t - 2) + ff_blocks(t - 1)
        ff_finish([jnp.where(i == 0, n_seg + j, s) for j, s in enumerate(pending)])
        memory = mem[...]
        for j in range(2):
            h = jnp.concatenate([nrm[seg_rows(t + j), :], nrm[seg_rows(t + j - LAG), :],
                                 memory.astype(BF16)], axis=0)
            memory, ff_in = fused_step(t + j, attention_stages(h, fill2, HEAD_GROUP), ff_in,
                                       slice(2 * j * seg, 2 * (j + 1) * seg),
                                       with_tail=j == 1, lead=1 - j)
        mem[...] = memory
        return carry

    def edge_step(s=None, layer=None, ff_segments=None, rider_tokens=None, rider_rows=None):
        ff_rows = slice(0, 2 * seg)
        chunks = iter(range(n_chunks) if ff_segments else ())
        if ff_segments:
            ff_in = jnp.concatenate([nrm[seg_rows(f), :] for f in ff_segments], axis=0)
        if s is not None:
            mem_rows = slice(layer * n_mem, (layer + 1) * n_mem)
            tokens = nrm[seg_rows(s), :].astype(F32)
            if rider_tokens is None:
                h = [tokens[n_mem:, :], mem[mem_rows, :]]
            else:
                h = [tokens, mem[mem_rows, :], rider_tokens]
            h = jnp.concatenate(h, axis=0).astype(BF16)

            def arrange(y, cols):
                if rider_tokens is None:
                    return jnp.concatenate([rider[rider_rows, cols], y], axis=0).astype(BF16)
                rider[rider_rows, cols] = y[seg + n_mem:, :]
                return y[0:seg + n_mem, :].astype(BF16)

            parts, projected = [], 0

            def project(stop):
                cols = slice(projected * head_dim, stop * head_dim)
                parts.append(_dot_nt(o_buf[0:seg + n_mem, cols], _as_bf16(wot[:, cols])))
                return stop

            for draining, finished in attention_stages(h, fill1, EDGE_GROUP, arrange):
                if draining and ff_segments:
                    gate_up(ff_in, next(chunks), ff_rows)
                elif draining and finished < n_heads:
                    projected = project(min(finished, projected + 3 * n_heads // 8))
        for c in chunks:
            gate_up(ff_in, c, ff_rows)
        if s is not None:
            project(n_heads)
            out = functools.reduce(jnp.add, parts)
        if ff_segments:
            ff_out = _dot_nt(h_buf[ff_rows, :], _as_bf16(w2t[...]))
        if s is not None:
            mem[mem_rows, :] = out[seg:, :]
            add_and_normalize(s, out[0:seg, :])
        for i, f in enumerate(ff_segments or ()):
            add_and_normalize(f, ff_out[i * seg:(i + 1) * seg, :])

    def head_step(s, carry):
        rows = _block(s, n_mem)
        edge_step(s, 0, rider_tokens=rider_in[rows, :], rider_rows=rows)
        return carry

    finished_blocks = (n_seg - LAG - 1) * seg // LANES
    tail_blocks = (finished_blocks - N_EARLY) // (LAG // 2)
    assert tail_blocks >= 0

    def tail_pair(i, carry):
        s = n_seg - LAG + 2 * i
        blocks = [N_EARLY + tail_blocks * i + j for j in range(tail_blocks)]
        for block in blocks:
            stage_output(block)
        following = nrm[seg_rows(s + 1), :].astype(F32)[0:n_mem, :]
        edge_step(s, 1, (jnp.where(i == 0, n_seg - 1, s - 2), s - 1), following, slice(0, n_mem))
        for block in blocks:
            out_copy(block).start()
        edge_step(s + 1, 1, rider_rows=slice(0, n_mem))
        return carry

    rider_in[...] = nrm[seq - seg:seq, :].astype(F32)
    lax.fori_loop(0, LAG, head_step, 0)
    for copy in ff_copies:
        copy.wait()
    early[(N_EARLY - 1) * seg:, :] = rider[...].astype(BF16)
    edge_step(ff_segments=(0, 1))
    lax.fori_loop(0, (first_early - LAG) // 2, fused_pair, 0)
    lax.fori_loop(first_early, n_seg, early_step, 0)
    ff_finish(ff_blocks(n_seg - 2) + ff_blocks(n_seg - 1))
    lax.fori_loop(0, LAG // 2, tail_pair, 0)
    edge_step(ff_segments=(n_seg - 2, n_seg - 1))
    for block in range(N_EARLY + tail_blocks * (LAG // 2), n_blocks):
        stage_output(block)
        out_copy(block).start()
    for block in range(n_blocks):
        out_copy(block).wait()


@functools.partial(jax.jit, static_argnames=("A_seg_len",))
def pallas_interleave_layers__memory_aug_recurrent_mem_tr__glu_gated_swiglu__prompt_kernel(
    A_x: jax.Array,
    A_mem0: jax.Array,
    A_Wq: jax.Array,
    A_Wk: jax.Array,
    A_Wv: jax.Array,
    A_Wo: jax.Array,
    A_seg_len: int,
    B_x: jax.Array,
    B_w1: jax.Array,
    B_w3: jax.Array,
    B_w2: jax.Array,
):
    del B_x
    batch, seq, d_model = A_x.shape
    n_mem = A_mem0.shape[1]
    _, n_heads, head_dim = A_Wq.shape
    d_ff = B_w1.shape[1]
    seg = int(A_seg_len)
    assert batch == 1 and seq % LANES == 0 and seq % seg == 0 and head_dim == LANES
    assert d_ff % FF_CHUNK == 0 and n_heads % HEAD_GROUP == 0 and N_EARLY % 2 == 0 and LAG == 4 and LAG * n_mem == seg
    rows = 2 * (seg + n_mem)

    any_spec = pl.BlockSpec(memory_space=pl.ANY)
    out_t = pl.pallas_call(
        functools.partial(_kernel, seg=seg, n_mem=n_mem, n_heads=n_heads, head_dim=head_dim),
        out_shape=jax.ShapeDtypeStruct((d_model, seq), A_x.dtype),
        in_specs=[any_spec, pl.BlockSpec(memory_space=pltpu.VMEM)] + [any_spec] * 7,
        out_specs=any_spec,
        scratch_shapes=[
            pltpu.VMEM((d_model, seq), BF16),
            pltpu.VMEM((3, n_heads // 2, d_model, head_dim), jnp.uint32),
            pltpu.VMEM((N_EARLY * seg, 3 * n_heads * head_dim), BF16),
            pltpu.VMEM((seg, d_model), F32),
            pltpu.VMEM((seg, 3 * n_heads * head_dim), F32),
            pltpu.VMEM((d_model // 2, 3 * n_heads * head_dim), jnp.uint32),
            pltpu.VMEM((d_model // 2, n_heads * head_dim), jnp.uint32),
            pltpu.VMEM((d_model // 2, d_ff), jnp.uint32),
            pltpu.VMEM((d_model // 2, d_ff), jnp.uint32),
            pltpu.VMEM((d_model // 2, d_ff), jnp.uint32),
            pltpu.VMEM((seq + 4 * seg, d_model), F32),
            pltpu.VMEM((seq + 4 * seg, d_model), BF16),
            pltpu.VMEM((2 * n_mem, d_model), F32),
            pltpu.VMEM((rows, n_heads * head_dim), BF16),
            pltpu.VMEM((4 * seg, d_ff), BF16),
            pltpu.VMEM((4 * seg, d_model // LANES * LANES), F32),
            pltpu.VMEM((d_model % LANES, 4 * seg), F32),
            pltpu.VMEM((rows // 2, rows // 2), F32),
            pltpu.VMEM((rows, rows), F32),
            pltpu.SemaphoreType.DMA((seq // LANES,)),
            pltpu.SemaphoreType.DMA((3, n_heads // 2)),
            pltpu.SemaphoreType.DMA((n_heads,)),
            pltpu.SemaphoreType.DMA((3,)),
            pltpu.SemaphoreType.DMA((seq // LANES,)),
        ],
        compiler_params=pltpu.CompilerParams(vmem_limit_bytes=100 * 1024 * 1024),
    )(
        A_x[0].T,
        A_mem0[0],
        A_Wq,
        A_Wk,
        A_Wv,
        jnp.transpose(A_Wo, (0, 2, 1)),
        B_w1,
        B_w3,
        B_w2.T,
    )
    return out_t.T[None]
```

```python
import functools
import math

import jax
import jax.numpy as jnp
from jax import lax
import jax.experimental.pallas as pl
import jax.experimental.pallas.tpu as pltpu

F32 = jnp.float32
BF16 = jnp.bfloat16
LANES = 128
LAG = 4
HEAD_GROUP = 2
EDGE_GROUP = 4
N_EARLY = 12
FF_CHUNK = 512
COPY_WINDOW = 3
LN_EPS = 1e-5
MASK_FILL = -1000000000.0
LOG2E = math.log2(math.e)
NT_DIMS = (((1,), (1,)), ((), ()))


def _dot(a, b):
    return jnp.dot(a, b, preferred_element_type=F32)


def _dot_nt(a, b):
    return lax.dot_general(a, b, NT_DIMS, preferred_element_type=F32)


def _as_bf16(words):
    return pltpu.bitcast(words, BF16)


def _block(index, size):
    start = index * size
    return pl.ds(start if isinstance(index, int) else pl.multiple_of(start, size), size)


def _layernorm(x):
    mean = jnp.mean(x, axis=-1, keepdims=True)
    cen = x - mean
    var = jnp.mean(cen * cen, axis=-1, keepdims=True)
    return cen * lax.rsqrt(var + LN_EPS)


def _mask_fill(n_streams, seg, n_mem):
    rows = n_streams * (seg + n_mem)

    def stream_and_pos(i):
        is_mem = i >= n_streams * seg
        j = i - n_streams * seg
        stream = jnp.where(is_mem, j // n_mem, i // seg)
        pos = jnp.where(is_mem, j % n_mem, n_mem + i % seg)
        return stream, pos

    q_stream, q_pos = stream_and_pos(lax.broadcasted_iota(jnp.int32, (rows, rows), 0))
    k_stream, k_pos = stream_and_pos(lax.broadcasted_iota(jnp.int32, (rows, rows), 1))
    visible = (q_pos < n_mem) | (q_pos >= k_pos)
    fill = jnp.where(visible, 0.0, MASK_FILL * LOG2E).astype(F32)
    return jnp.where(q_stream == k_stream, fill, -jnp.inf)


def _kernel(xt_hbm, mem0_ref, wq_hbm, wk_hbm, wv_hbm, wot_hbm, w1_hbm, w3_hbm, w2t_hbm,
            out_hbm,
            xt_buf, stage, early, rider_in, rider, wqkv, wot, w1, w3, w2t, res, nrm, mem, o_buf, h_buf, ff_main, ff_tail,
            fill1, fill2, sem_x, sem_qkv, sem_o, sem_ff, sem_out,
            *, seg, n_mem, n_heads, head_dim):
    d_model, seq = xt_buf.shape
    d_ff = w1.shape[1]
    d_main = d_model // LANES * LANES
    n_seg = seq // seg
    n_pairs = n_heads // 2
    n_chunks = d_ff // FF_CHUNK
    score_scale = head_dim ** -0.5 * LOG2E
    head_cols = 3 * head_dim

    n_blocks = seq // LANES
    first_early = n_seg - N_EARLY
    late_blocks = first_early * seg // LANES

    def x_copy(block):
        tok = _block(block, LANES)
        return pltpu.make_async_copy(xt_hbm.at[:, tok], xt_buf.at[:, tok], sem_x.at[block])

    def qkv_copy(pair, which):
        src = (wq_hbm, wk_hbm, wv_hbm)[which].bitcast(jnp.uint32)
        return pltpu.make_async_copy(src.at[:, pair, :], stage.at[which, pair],
                                     sem_qkv.at[which, pair])

    def wo_copy(head):
        return pltpu.make_async_copy(wot_hbm.bitcast(jnp.uint32).at[head],
                                     wot.at[:, pl.ds(head * head_dim, head_dim)], sem_o.at[head])

    ff_copies = [pltpu.make_async_copy(src.bitcast(jnp.uint32), dst, sem_ff.at[i])
                 for i, (src, dst) in enumerate(((w1_hbm, w1), (w3_hbm, w3), (w2t_hbm, w2t)))]

    for block in range(late_blocks, n_blocks):
        x_copy(block).start()
    for which in range(3):
        qkv_copy(0, which).start()

    fill1[...] = _mask_fill(1, seg, n_mem)
    fill2[...] = _mask_fill(2, seg, n_mem)
    mem0 = mem0_ref[...].astype(F32)
    mem[0:n_mem, :] = mem0
    mem[n_mem:2 * n_mem, :] = mem0

    ff_main[...] = jnp.zeros(ff_main.shape, F32)
    ff_tail[...] = jnp.zeros(ff_tail.shape, F32)

    for block in range(late_blocks, n_blocks):
        x_copy(block).wait()
    for pair in range(1, COPY_WINDOW):
        for which in range(3):
            qkv_copy(pair, which).start()

    def load_tokens(src_block, dst_block):
        x = xt_buf[:, _block(src_block, LANES)].astype(F32).T
        rows = _block(dst_block, LANES)
        res[rows, :] = x
        nrm[rows, :] = _layernorm(x).astype(BF16)

    for block in range(late_blocks, n_blocks):
        load_tokens(block, block)

    def prepare_pair(pair, carry):
        ahead = pair + COPY_WINDOW
        block = pair - (n_pairs - late_blocks)

        @pl.when(ahead < n_pairs)
        def _():
            for which in range(3):
                qkv_copy(ahead, which).start()

        @pl.when(ahead == n_pairs)
        def _():
            for head in range(n_heads):
                wo_copy(head).start()

        @pl.when(pair < late_blocks)
        def _():
            x_copy(pair).start()

        @pl.when(block >= 0)
        def _():
            x_copy(block).wait()

        for which in range(3):
            qkv_copy(pair, which).wait()
        words = [stage[which, pair] for which in range(3)]
        even = [lax.bitcast_convert_type(w << 16, F32) for w in words]
        odd = [lax.bitcast_convert_type(w & jnp.uint32(0xFFFF0000), F32) for w in words]
        w_pair = jnp.concatenate([w.astype(BF16) for w in even + odd], axis=1)
        cols = _block(pair, 2 * head_cols)
        early[0:(N_EARLY - 1) * seg, cols] = _dot(
            nrm[first_early * seg:seq - seg, :], w_pair).astype(BF16)
        wqkv[:, cols] = pltpu.bitcast(w_pair, jnp.uint32)
        load_tokens(jnp.where(block < 0, late_blocks, block), jnp.where(block < 0, n_blocks, block))
        return carry

    lax.fori_loop(0, n_pairs, prepare_pair, 0)
    for head in range(n_heads):
        wo_copy(head).wait()
    for copy in ff_copies:
        copy.start()

    def seg_rows(s):
        return _block(s, seg)

    def add_and_normalize(s, delta):
        x = res[seg_rows(s), :] + delta
        normalized = _layernorm(x).astype(BF16)
        res[seg_rows(s), :] = x
        nrm[seg_rows(s), :] = normalized
        return normalized

    def attention_stages(h, fill_ref, group, arrange=lambda y, cols: y.astype(BF16)):
        rows = fill_ref.shape[0]
        n_groups = n_heads // group
        qkv, probs = {}, {}
        for g in range(n_groups + 2):
            if g < n_groups:
                cols = slice(g * group * head_cols, (g + 1) * group * head_cols)
                qkv[g] = arrange(_dot(h, _as_bf16(wqkv[:, cols])), cols)
            if 0 <= g - 1 < n_groups:
                y = qkv[g - 1]
                probs[g - 1] = []
                for i in range(group):
                    q = y[:, i * head_cols:i * head_cols + head_dim]
                    k = y[:, i * head_cols + head_dim:i * head_cols + 2 * head_dim]
                    fill = fill_ref[...]
                    s = jnp.where(fill == 0.0, _dot_nt(q, k) * score_scale, fill)
                    e = jnp.exp2(s - jnp.max(s, axis=-1, keepdims=True))
                    p = e * (1.0 / jnp.sum(e, axis=-1, keepdims=True))
                    probs[g - 1].append(p.astype(BF16))
            if 0 <= g - 2 < n_groups:
                y = qkv.pop(g - 2)
                for i, p in enumerate(probs.pop(g - 2)):
                    v = y[:, i * head_cols + 2 * head_dim:(i + 1) * head_cols]
                    head = (g - 2) * group + i
                    o_buf[0:rows, head * head_dim:(head + 1) * head_dim] = _dot(p, v).astype(BF16)
            yield g >= n_groups - 1, max(g - 1, 0) * group

    def project_main(act, wt_ref):
        return _dot_nt(act, _as_bf16(wt_ref[0:d_main // 2, :]))

    def project_tail(act, wt_ref):
        return _dot_nt(_as_bf16(wt_ref[d_main // 2:, :]), act)

    def gate_up(hf, c, rows):
        cols = slice(c * FF_CHUNK, (c + 1) * FF_CHUNK)
        gate = _dot(hf, _as_bf16(w1[:, cols]))
        up = _dot(hf, _as_bf16(w3[:, cols]))
        h_buf[rows, cols] = (gate * (1.0 / (1.0 + jnp.exp(-gate))) * up).astype(BF16)

    def ff_input(t):
        sa, sb = ff_blocks(t)
        return jnp.concatenate([nrm[seg_rows(sa), :], nrm[seg_rows(sb), :]], axis=0)

    def ff_finish(segments):
        out = jnp.concatenate([ff_main[...], ff_tail[...].T], axis=1)
        for i, s in enumerate(segments):
            add_and_normalize(s, out[i * seg:(i + 1) * seg, :])

    def ff_blocks(t):
        if isinstance(t, int):
            return t - 1, t - LAG - 1
        return t - 1, jnp.where(t == LAG, t - 2, t - LAG - 1)

    def out_copy(block):
        tok = _block(block, LANES)
        return pltpu.make_async_copy(xt_buf.at[:, tok], out_hbm.at[:, tok], sem_out.at[block])

    def stage_output(block):
        tok = _block(block, LANES)
        xt_buf[:, tok] = res[tok, :].T.astype(BF16)

    def fused_step(t, stages, ff_in, ff_rows, with_tail, lead=0):
        chunks = iter(range(n_chunks))
        for _ in range(lead):
            gate_up(ff_in, next(chunks), ff_rows)
        for draining, _ in stages:
            if draining:
                gate_up(ff_in, next(chunks), ff_rows)
        for c in chunks:
            gate_up(ff_in, c, ff_rows)
        heads = o_buf[...]
        tail = project_tail(heads, wot)
        out = jnp.concatenate([project_main(heads, wot), tail.T], axis=1)
        if with_tail:
            ff_tail[...] = project_tail(h_buf[...], w2t)
        ff_main[ff_rows, :] = project_main(h_buf[ff_rows, :], w2t)
        next_in = jnp.concatenate([add_and_normalize(t, out[0:seg, :]),
                                   add_and_normalize(t - LAG, out[seg:2 * seg, :])], axis=0)
        return out[2 * seg:, :], next_in

    def early_step(t, carry):
        odd = t % 2
        ff_in = ff_input(t)
        pending = ff_blocks(t - 2) + ff_blocks(t - 1)
        ff_finish([jnp.where(odd == 1, n_seg + j, s) for j, s in enumerate(pending)])
        stage_output(t - first_early)
        h = jnp.concatenate([nrm[seg_rows(t - LAG), :], mem[...].astype(BF16)], axis=0)

        def prepend_early(y, cols):
            return jnp.concatenate([early[seg_rows(t - first_early), cols], y.astype(BF16)], axis=0)

        stages = attention_stages(h, fill2, HEAD_GROUP, prepend_early)
        ff_rows = _block(odd, 2 * seg)
        mem[...], _ = fused_step(t, stages, ff_in, ff_rows, with_tail=False, lead=1)
        out_copy(t - first_early).start()

        @pl.when(odd == 1)
        def _():
            ff_tail[...] = project_tail(h_buf[...], w2t)

        return carry

    def fused_pair(i, carry):
        t = LAG + 2 * i
        ff_in = ff_input(t)
        pending = ff_blocks(t - 2) + ff_blocks(t - 1)
        ff_finish([jnp.where(i == 0, n_seg + j, s) for j, s in enumerate(pending)])
        memory = mem[...]
        for j in range(2):
            h = jnp.concatenate([nrm[seg_rows(t + j), :], nrm[seg_rows(t + j - LAG), :],
                                 memory.astype(BF16)], axis=0)
            memory, ff_in = fused_step(t + j, attention_stages(h, fill2, HEAD_GROUP), ff_in,
                                       slice(2 * j * seg, 2 * (j + 1) * seg),
                                       with_tail=j == 1, lead=1 - j)
        mem[...] = memory
        return carry

    def edge_step(s=None, layer=None, ff_segments=None, rider_tokens=None, rider_rows=None,
                  last=False):
        ff_rows = slice(0, 2 * seg)
        chunks = iter(range(n_chunks) if ff_segments else ())
        if ff_segments:
            ff_in = jnp.concatenate([nrm[seg_rows(f), :] for f in ff_segments], axis=0)
        if s is not None:
            mem_rows = slice(layer * n_mem, (layer + 1) * n_mem)
            tokens = nrm[seg_rows(s), :].astype(F32)
            if rider_tokens is None:
                h = [tokens[n_mem:, :], mem[mem_rows, :]]
            else:
                h = [tokens, mem[mem_rows, :], rider_tokens]
            h = jnp.concatenate(h, axis=0).astype(BF16)

            def arrange(y, cols):
                if rider_tokens is None:
                    return jnp.concatenate([rider[rider_rows, cols], y], axis=0).astype(BF16)
                rider[rider_rows, cols] = y[seg + n_mem:, :]
                return y[0:seg + n_mem, :].astype(BF16)

            parts, projected = [], 0

            def project(stop):
                cols = slice(projected * head_dim, stop * head_dim)
                parts.append(_dot_nt(o_buf[0:seg + n_mem, cols], _as_bf16(wot[:, cols])))
                return stop

            for draining, finished in attention_stages(h, fill1, EDGE_GROUP, arrange):
                if draining and ff_segments:
                    gate_up(ff_in, next(chunks), ff_rows)
                elif draining and finished < n_heads:
                    projected = project(min(finished, projected + 3 * n_heads // 8))
        for c in chunks:
            gate_up(ff_in, c, ff_rows)
        if s is not None:
            project(n_heads)
            out = functools.reduce(jnp.add, parts)
        if ff_segments:
            ff_out = _dot_nt(h_buf[ff_rows, :], _as_bf16(w2t[...]))
        if s is not None:
            mem[mem_rows, :] = out[seg:, :]
            add_and_normalize(s, out[0:seg, :])
        for i, f in enumerate(ff_segments or ()):
            if last:
                res[seg_rows(f), :] += ff_out[i * seg:(i + 1) * seg, :]
            else:
                add_and_normalize(f, ff_out[i * seg:(i + 1) * seg, :])

    def head_step(s, carry):
        rows = _block(s, n_mem)
        edge_step(s, 0, rider_tokens=rider_in[rows, :], rider_rows=rows)
        return carry

    finished_blocks = (n_seg - LAG - 1) * seg // LANES
    tail_blocks = (finished_blocks - N_EARLY) // (LAG // 2)
    assert tail_blocks >= 0

    def tail_pair(i, carry):
        s = n_seg - LAG + 2 * i
        blocks = [N_EARLY + tail_blocks * i + j for j in range(tail_blocks)]
        for block in blocks:
            stage_output(block)
        following = nrm[seg_rows(s + 1), :].astype(F32)[0:n_mem, :]
        edge_step(s, 1, (jnp.where(i == 0, n_seg - 1, s - 2), s - 1), following, slice(0, n_mem))
        for block in blocks:
            out_copy(block).start()
        edge_step(s + 1, 1, rider_rows=slice(0, n_mem))
        return carry

    rider_in[...] = nrm[seq - seg:seq, :].astype(F32)
    lax.fori_loop(0, LAG, head_step, 0)
    for copy in ff_copies:
        copy.wait()
    early[(N_EARLY - 1) * seg:, :] = rider[...].astype(BF16)
    edge_step(ff_segments=(0, 1))
    lax.fori_loop(0, (first_early - LAG) // 2, fused_pair, 0)
    lax.fori_loop(first_early, n_seg, early_step, 0)
    ff_finish(ff_blocks(n_seg - 2) + ff_blocks(n_seg - 1))
    lax.fori_loop(0, LAG // 2, tail_pair, 0)
    remaining = range(N_EARLY + tail_blocks * (LAG // 2), n_blocks)
    for block in remaining[:-1]:
        stage_output(block)
    edge_step(ff_segments=(n_seg - 2, n_seg - 1), last=True)
    stage_output(remaining[-1])
    for block in remaining:
        out_copy(block).start()
    for block in range(n_blocks):
        out_copy(block).wait()


@functools.partial(jax.jit, static_argnames=("A_seg_len",))
def pallas_interleave_layers__memory_aug_recurrent_mem_tr__glu_gated_swiglu__prompt_kernel(
    A_x: jax.Array,
    A_mem0: jax.Array,
    A_Wq: jax.Array,
    A_Wk: jax.Array,
    A_Wv: jax.Array,
    A_Wo: jax.Array,
    A_seg_len: int,
    B_x: jax.Array,
    B_w1: jax.Array,
    B_w3: jax.Array,
    B_w2: jax.Array,
):
    del B_x
    batch, seq, d_model = A_x.shape
    n_mem = A_mem0.shape[1]
    _, n_heads, head_dim = A_Wq.shape
    d_ff = B_w1.shape[1]
    seg = int(A_seg_len)
    assert batch == 1 and seq % LANES == 0 and seq % seg == 0 and head_dim == LANES
    assert d_ff % FF_CHUNK == 0 and n_heads % HEAD_GROUP == 0 and N_EARLY % 2 == 0 and LAG == 4 and LAG * n_mem == seg
    rows = 2 * (seg + n_mem)

    any_spec = pl.BlockSpec(memory_space=pl.ANY)
    out_t = pl.pallas_call(
        functools.partial(_kernel, seg=seg, n_mem=n_mem, n_heads=n_heads, head_dim=head_dim),
        out_shape=jax.ShapeDtypeStruct((d_model, seq), A_x.dtype),
        in_specs=[any_spec, pl.BlockSpec(memory_space=pltpu.VMEM)] + [any_spec] * 7,
        out_specs=any_spec,
        scratch_shapes=[
            pltpu.VMEM((d_model, seq), BF16),
            pltpu.VMEM((3, n_heads // 2, d_model, head_dim), jnp.uint32),
            pltpu.VMEM((N_EARLY * seg, 3 * n_heads * head_dim), BF16),
            pltpu.VMEM((seg, d_model), F32),
            pltpu.VMEM((seg, 3 * n_heads * head_dim), F32),
            pltpu.VMEM((d_model // 2, 3 * n_heads * head_dim), jnp.uint32),
            pltpu.VMEM((d_model // 2, n_heads * head_dim), jnp.uint32),
            pltpu.VMEM((d_model // 2, d_ff), jnp.uint32),
            pltpu.VMEM((d_model // 2, d_ff), jnp.uint32),
            pltpu.VMEM((d_model // 2, d_ff), jnp.uint32),
            pltpu.VMEM((seq + 4 * seg, d_model), F32),
            pltpu.VMEM((seq + 4 * seg, d_model), BF16),
            pltpu.VMEM((2 * n_mem, d_model), F32),
            pltpu.VMEM((rows, n_heads * head_dim), BF16),
            pltpu.VMEM((4 * seg, d_ff), BF16),
            pltpu.VMEM((4 * seg, d_model // LANES * LANES), F32),
            pltpu.VMEM((d_model % LANES, 4 * seg), F32),
            pltpu.VMEM((rows // 2, rows // 2), F32),
            pltpu.VMEM((rows, rows), F32),
            pltpu.SemaphoreType.DMA((seq // LANES,)),
            pltpu.SemaphoreType.DMA((3, n_heads // 2)),
            pltpu.SemaphoreType.DMA((n_heads,)),
            pltpu.SemaphoreType.DMA((3,)),
            pltpu.SemaphoreType.DMA((seq // LANES,)),
        ],
        compiler_params=pltpu.CompilerParams(vmem_limit_bytes=100 * 1024 * 1024),
    )(
        A_x[0].T,
        A_mem0[0],
        A_Wq,
        A_Wk,
        A_Wv,
        jnp.transpose(A_Wo, (0, 2, 1)),
        B_w1,
        B_w3,
        B_w2.T,
    )
    return out_t.T[None]
```

```python
import functools
import math

import jax
import jax.numpy as jnp
from jax import lax
import jax.experimental.pallas as pl
import jax.experimental.pallas.tpu as pltpu

F32 = jnp.float32
BF16 = jnp.bfloat16
LANES = 128
LAG = 4
HEAD_GROUP = 2
EDGE_GROUP = 4
N_EARLY = 12
FF_CHUNK = 512
COPY_WINDOW = 3
LN_EPS = 1e-5
MASK_FILL = -1000000000.0
LOG2E = math.log2(math.e)
NT_DIMS = (((1,), (1,)), ((), ()))


def _dot(a, b):
    return jnp.dot(a, b, preferred_element_type=F32)


def _dot_nt(a, b):
    return lax.dot_general(a, b, NT_DIMS, preferred_element_type=F32)


def _as_bf16(words):
    return pltpu.bitcast(words, BF16)


def _block(index, size):
    start = index * size
    return pl.ds(start if isinstance(index, int) else pl.multiple_of(start, size), size)


def _layernorm(x):
    mean = jnp.mean(x, axis=-1, keepdims=True)
    cen = x - mean
    var = jnp.mean(cen * cen, axis=-1, keepdims=True)
    return cen * lax.rsqrt(var + LN_EPS)


def _mask_fill(n_streams, seg, n_mem):
    rows = n_streams * (seg + n_mem)

    def stream_and_pos(i):
        is_mem = i >= n_streams * seg
        j = i - n_streams * seg
        stream = jnp.where(is_mem, j // n_mem, i // seg)
        pos = jnp.where(is_mem, j % n_mem, n_mem + i % seg)
        return stream, pos

    q_stream, q_pos = stream_and_pos(lax.broadcasted_iota(jnp.int32, (rows, rows), 0))
    k_stream, k_pos = stream_and_pos(lax.broadcasted_iota(jnp.int32, (rows, rows), 1))
    visible = (q_pos < n_mem) | (q_pos >= k_pos)
    fill = jnp.where(visible, 0.0, MASK_FILL * LOG2E).astype(F32)
    return jnp.where(q_stream == k_stream, fill, -jnp.inf)


def _kernel(xt_hbm, mem0_ref, wq_hbm, wk_hbm, wv_hbm, wot_hbm, w1_hbm, w3_hbm, w2t_hbm,
            out_hbm,
            xt_buf, stage, early, rider_in, rider, wqkv, wot, w1, w3, w2t, res, nrm, mem,
            o_buf, h_buf, ff_main, ff_tail, fill1, fill2,
            sem_x, sem_qkv, sem_o, sem_ff, sem_out,
            *, seg, n_mem, n_heads, head_dim):
    d_model, seq = xt_buf.shape
    d_ff = w1.shape[1]
    d_main = d_model // LANES * LANES
    n_seg = seq // seg
    n_pairs = n_heads // 2
    n_chunks = d_ff // FF_CHUNK
    score_scale = head_dim ** -0.5 * LOG2E
    head_cols = 3 * head_dim

    n_blocks = seq // LANES
    first_early = n_seg - N_EARLY
    late_blocks = first_early * seg // LANES

    def x_copy(block):
        tok = _block(block, LANES)
        return pltpu.make_async_copy(xt_hbm.at[:, tok], xt_buf.at[:, tok], sem_x.at[block])

    def qkv_copy(pair, which):
        src = (wq_hbm, wk_hbm, wv_hbm)[which].bitcast(jnp.uint32)
        return pltpu.make_async_copy(src.at[:, pair, :], stage.at[which, pair],
                                     sem_qkv.at[which, pair])

    def wo_copy(head):
        return pltpu.make_async_copy(wot_hbm.bitcast(jnp.uint32).at[head],
                                     wot.at[:, pl.ds(head * head_dim, head_dim)], sem_o.at[head])

    ff_copies = [pltpu.make_async_copy(src.bitcast(jnp.uint32), dst, sem_ff.at[i])
                 for i, (src, dst) in enumerate(((w1_hbm, w1), (w3_hbm, w3), (w2t_hbm, w2t)))]

    for block in range(late_blocks, n_blocks):
        x_copy(block).start()
    for which in range(3):
        qkv_copy(0, which).start()

    fill1[...] = _mask_fill(1, seg, n_mem)
    fill2[...] = _mask_fill(2, seg, n_mem)
    mem0 = mem0_ref[...].astype(F32)
    mem[0:n_mem, :] = mem0
    mem[n_mem:2 * n_mem, :] = mem0

    ff_main[...] = jnp.zeros(ff_main.shape, F32)
    ff_tail[...] = jnp.zeros(ff_tail.shape, F32)

    for block in range(late_blocks, n_blocks):
        x_copy(block).wait()
    for pair in range(1, COPY_WINDOW):
        for which in range(3):
            qkv_copy(pair, which).start()

    def load_tokens(src_block, dst_block):
        x = xt_buf[:, _block(src_block, LANES)].astype(F32).T
        rows = _block(dst_block, LANES)
        res[rows, :] = x
        nrm[rows, :] = _layernorm(x).astype(BF16)

    for block in range(late_blocks, n_blocks):
        load_tokens(block, block)

    def prepare_pair(pair, carry):
        ahead = pair + COPY_WINDOW
        block = pair - (n_pairs - late_blocks)

        @pl.when(ahead < n_pairs)
        def _():
            for which in range(3):
                qkv_copy(ahead, which).start()

        @pl.when(ahead == n_pairs)
        def _():
            for head in range(n_heads):
                wo_copy(head).start()

        @pl.when(pair < late_blocks)
        def _():
            x_copy(pair).start()

        @pl.when(block >= 0)
        def _():
            x_copy(block).wait()

        for which in range(3):
            qkv_copy(pair, which).wait()
        words = [stage[which, pair] for which in range(3)]
        even = [lax.bitcast_convert_type(w << 16, F32) for w in words]
        odd = [lax.bitcast_convert_type(w & jnp.uint32(0xFFFF0000), F32) for w in words]
        w_pair = jnp.concatenate([w.astype(BF16) for w in even + odd], axis=1)
        cols = _block(pair, 2 * head_cols)
        early[0:(N_EARLY - 1) * seg, cols] = _dot(
            nrm[first_early * seg:seq - seg, :], w_pair).astype(BF16)
        wqkv[:, cols] = pltpu.bitcast(w_pair, jnp.uint32)
        load_tokens(jnp.where(block < 0, late_blocks, block), jnp.where(block < 0, n_blocks, block))
        return carry

    lax.fori_loop(0, n_pairs, prepare_pair, 0)
    for head in range(n_heads):
        wo_copy(head).wait()
    for copy in ff_copies:
        copy.start()

    def seg_rows(s):
        return _block(s, seg)

    def add_and_normalize(s, delta):
        x = res[seg_rows(s), :] + delta
        normalized = _layernorm(x).astype(BF16)
        res[seg_rows(s), :] = x
        nrm[seg_rows(s), :] = normalized
        return normalized

    def attention_stages(h, fill_ref, group, arrange=lambda y, cols: y.astype(BF16)):
        rows = fill_ref.shape[0]
        n_groups = n_heads // group
        qkv, probs = {}, {}
        for g in range(n_groups + 2):
            if g < n_groups:
                cols = slice(g * group * head_cols, (g + 1) * group * head_cols)
                qkv[g] = arrange(_dot(h, _as_bf16(wqkv[:, cols])), cols)
            if 0 <= g - 1 < n_groups:
                y = qkv[g - 1]
                probs[g - 1] = []
                for i in range(group):
                    q = y[:, i * head_cols:i * head_cols + head_dim]
                    k = y[:, i * head_cols + head_dim:i * head_cols + 2 * head_dim]
                    fill = fill_ref[...]
                    s = jnp.where(fill == 0.0, _dot_nt(q, k) * score_scale, fill)
                    e = jnp.exp2(s - jnp.max(s, axis=-1, keepdims=True))
                    p = e * (1.0 / jnp.sum(e, axis=-1, keepdims=True))
                    probs[g - 1].append(p.astype(BF16))
            if 0 <= g - 2 < n_groups:
                y = qkv.pop(g - 2)
                for i, p in enumerate(probs.pop(g - 2)):
                    v = y[:, i * head_cols + 2 * head_dim:(i + 1) * head_cols]
                    head = (g - 2) * group + i
                    o_buf[0:rows, head * head_dim:(head + 1) * head_dim] = _dot(p, v).astype(BF16)
            yield g >= n_groups - 1, max(g - 1, 0) * group

    def project_main(act, wt_ref):
        return _dot_nt(act, _as_bf16(wt_ref[0:d_main // 2, :]))

    def project_tail(act, wt_ref):
        return _dot_nt(_as_bf16(wt_ref[d_main // 2:, :]), act)

    def gate_up(hf, c, rows):
        cols = slice(c * FF_CHUNK, (c + 1) * FF_CHUNK)
        gate = _dot(hf, _as_bf16(w1[:, cols]))
        up = _dot(hf, _as_bf16(w3[:, cols]))
        h_buf[rows, cols] = (gate * (1.0 / (1.0 + jnp.exp(-gate))) * up).astype(BF16)

    def ff_input(t):
        sa, sb = ff_blocks(t)
        return jnp.concatenate([nrm[seg_rows(sa), :], nrm[seg_rows(sb), :]], axis=0)

    def ff_finish(segments):
        out = jnp.concatenate([ff_main[...], ff_tail[...].T], axis=1)
        for i, s in enumerate(segments):
            add_and_normalize(s, out[i * seg:(i + 1) * seg, :])

    def ff_blocks(t):
        if isinstance(t, int):
            return t - 1, t - LAG - 1
        return t - 1, jnp.where(t == LAG, t - 2, t - LAG - 1)

    def out_copy(block):
        tok = _block(block, LANES)
        return pltpu.make_async_copy(xt_buf.at[:, tok], out_hbm.at[:, tok], sem_out.at[block])

    def stage_output(block):
        tok = _block(block, LANES)
        xt_buf[:, tok] = res[tok, :].T.astype(BF16)

    def fused_step(t, stages, ff_in, ff_rows, with_tail, lead=0):
        chunks = iter(range(n_chunks))
        for _ in range(lead):
            gate_up(ff_in, next(chunks), ff_rows)
        for draining, _ in stages:
            if draining:
                gate_up(ff_in, next(chunks), ff_rows)
        for c in chunks:
            gate_up(ff_in, c, ff_rows)
        heads = o_buf[...]
        tail = project_tail(heads, wot)
        out = jnp.concatenate([project_main(heads, wot), tail.T], axis=1)
        if with_tail:
            ff_tail[...] = project_tail(h_buf[...], w2t)
        ff_main[ff_rows, :] = project_main(h_buf[ff_rows, :], w2t)
        next_in = jnp.concatenate([add_and_normalize(t, out[0:seg, :]),
                                   add_and_normalize(t - LAG, out[seg:2 * seg, :])], axis=0)
        return out[2 * seg:, :], next_in

    def early_step(t, carry):
        odd = t % 2
        ff_in = ff_input(t)
        pending = ff_blocks(t - 2) + ff_blocks(t - 1)
        ff_finish([jnp.where(odd == 1, n_seg + j, s) for j, s in enumerate(pending)])
        stage_output(t - first_early)
        h = jnp.concatenate([nrm[seg_rows(t - LAG), :], mem[...].astype(BF16)], axis=0)

        def prepend_early(y, cols):
            return jnp.concatenate([early[seg_rows(t - first_early), cols], y.astype(BF16)], axis=0)

        stages = attention_stages(h, fill2, HEAD_GROUP, prepend_early)
        ff_rows = _block(odd, 2 * seg)
        mem[...], _ = fused_step(t, stages, ff_in, ff_rows, with_tail=False, lead=1)
        out_copy(t - first_early).start()

        @pl.when(odd == 1)
        def _():
            ff_tail[...] = project_tail(h_buf[...], w2t)

        return carry

    def fused_pair(i, carry):
        t = LAG + 2 * i
        ff_in = ff_input(t)
        pending = ff_blocks(t - 2) + ff_blocks(t - 1)
        ff_finish([jnp.where(i == 0, n_seg + j, s) for j, s in enumerate(pending)])
        memory = mem[...]
        for j in range(2):
            h = jnp.concatenate([nrm[seg_rows(t + j), :], nrm[seg_rows(t + j - LAG), :],
                                 memory.astype(BF16)], axis=0)
            memory, ff_in = fused_step(t + j, attention_stages(h, fill2, HEAD_GROUP), ff_in,
                                       slice(2 * j * seg, 2 * (j + 1) * seg),
                                       with_tail=j == 1, lead=1 - j)
        mem[...] = memory
        return carry

    def edge_step(s=None, layer=None, ff_segments=None, rider_tokens=None, rider_rows=None,
                  last=False):
        ff_rows = slice(0, 2 * seg)
        chunks = iter(range(n_chunks) if ff_segments else ())
        if ff_segments:
            ff_in = jnp.concatenate([nrm[seg_rows(f), :] for f in ff_segments], axis=0)
        if s is not None:
            mem_rows = slice(layer * n_mem, (layer + 1) * n_mem)
            tokens = nrm[seg_rows(s), :].astype(F32)
            if rider_tokens is None:
                h = [tokens[n_mem:, :], mem[mem_rows, :]]
            else:
                h = [tokens, mem[mem_rows, :], rider_tokens]
            h = jnp.concatenate(h, axis=0).astype(BF16)

            def arrange(y, cols):
                if rider_tokens is None:
                    return jnp.concatenate([rider[rider_rows, cols], y], axis=0).astype(BF16)
                rider[rider_rows, cols] = y[seg + n_mem:, :]
                return y[0:seg + n_mem, :].astype(BF16)

            parts, projected = [], 0

            def project(stop):
                cols = slice(projected * head_dim, stop * head_dim)
                parts.append(_dot_nt(o_buf[0:seg + n_mem, cols], _as_bf16(wot[:, cols])))
                return stop

            for draining, finished in attention_stages(h, fill1, EDGE_GROUP, arrange):
                if draining and ff_segments:
                    gate_up(ff_in, next(chunks), ff_rows)
                elif draining and finished < n_heads:
                    projected = project(min(finished, projected + 3 * n_heads // 8))
        for c in chunks:
            gate_up(ff_in, c, ff_rows)
        if s is not None:
            project(n_heads)
            out = functools.reduce(jnp.add, parts)
        if ff_segments:
            ff_out = _dot_nt(h_buf[ff_rows, :], _as_bf16(w2t[...]))
        if s is not None:
            mem[mem_rows, :] = out[seg:, :]
            add_and_normalize(s, out[0:seg, :])
        for i, f in enumerate(ff_segments or ()):
            if last:
                res[seg_rows(f), :] += ff_out[i * seg:(i + 1) * seg, :]
            else:
                add_and_normalize(f, ff_out[i * seg:(i + 1) * seg, :])

    def head_step(s, carry):
        rows = _block(s, n_mem)
        edge_step(s, 0, rider_tokens=rider_in[rows, :], rider_rows=rows)
        return carry

    finished_blocks = (n_seg - LAG - 1) * seg // LANES
    tail_blocks = (finished_blocks - N_EARLY) // (LAG // 2)
    assert tail_blocks >= 0

    def tail_pair(i, carry):
        s = n_seg - LAG + 2 * i
        blocks = [N_EARLY + tail_blocks * i + j for j in range(tail_blocks)]
        for block in blocks:
            stage_output(block)
        following = nrm[seg_rows(s + 1), :].astype(F32)[0:n_mem, :]
        edge_step(s, 1, (jnp.where(i == 0, n_seg - 1, s - 2), s - 1), following, slice(0, n_mem))
        for block in blocks:
            out_copy(block).start()
        edge_step(s + 1, 1, rider_rows=slice(0, n_mem))
        return carry

    rider_in[...] = nrm[seq - seg:seq, :].astype(F32)
    lax.fori_loop(0, LAG, head_step, 0)
    for copy in ff_copies:
        copy.wait()
    early[(N_EARLY - 1) * seg:, :] = rider[...].astype(BF16)
    edge_step(ff_segments=(0, 1))
    lax.fori_loop(0, (first_early - LAG) // 2, fused_pair, 0)
    lax.fori_loop(first_early, n_seg, early_step, 0)
    ff_finish(ff_blocks(n_seg - 2) + ff_blocks(n_seg - 1))
    lax.fori_loop(0, LAG // 2, tail_pair, 0)
    remaining = range(N_EARLY + tail_blocks * (LAG // 2), n_blocks)
    for block in remaining[:-1]:
        stage_output(block)
    edge_step(ff_segments=(n_seg - 2, n_seg - 1), last=True)
    stage_output(remaining[-1])
    for block in remaining:
        out_copy(block).start()
    for block in range(n_blocks):
        out_copy(block).wait()


@functools.partial(jax.jit, static_argnames=("A_seg_len",))
def pallas_interleave_layers__memory_aug_recurrent_mem_tr__glu_gated_swiglu__prompt_kernel(
    A_x: jax.Array,
    A_mem0: jax.Array,
    A_Wq: jax.Array,
    A_Wk: jax.Array,
    A_Wv: jax.Array,
    A_Wo: jax.Array,
    A_seg_len: int,
    B_x: jax.Array,
    B_w1: jax.Array,
    B_w3: jax.Array,
    B_w2: jax.Array,
):
    del B_x
    batch, seq, d_model = A_x.shape
    n_mem = A_mem0.shape[1]
    _, n_heads, head_dim = A_Wq.shape
    d_ff = B_w1.shape[1]
    seg = int(A_seg_len)
    assert batch == 1 and head_dim == LANES and seq % LANES == 0 and 4 * seg == LANES
    assert d_ff % FF_CHUNK == 0 and n_heads % EDGE_GROUP == 0 and d_model % LANES != 0
    assert LAG == 4 and LAG * n_mem == seg and N_EARLY % 4 == 0
    assert (seq // seg - N_EARLY) * seg // LANES < n_heads // 2
    rows = 2 * (seg + n_mem)

    any_spec = pl.BlockSpec(memory_space=pl.ANY)
    out_t = pl.pallas_call(
        functools.partial(_kernel, seg=seg, n_mem=n_mem, n_heads=n_heads, head_dim=head_dim),
        out_shape=jax.ShapeDtypeStruct((d_model, seq), A_x.dtype),
        in_specs=[any_spec, pl.BlockSpec(memory_space=pltpu.VMEM)] + [any_spec] * 7,
        out_specs=any_spec,
        scratch_shapes=[
            pltpu.VMEM((d_model, seq), BF16),
            pltpu.VMEM((3, n_heads // 2, d_model, head_dim), jnp.uint32),
            pltpu.VMEM((N_EARLY * seg, 3 * n_heads * head_dim), BF16),
            pltpu.VMEM((seg, d_model), F32),
            pltpu.VMEM((seg, 3 * n_heads * head_dim), F32),
            pltpu.VMEM((d_model // 2, 3 * n_heads * head_dim), jnp.uint32),
            pltpu.VMEM((d_model // 2, n_heads * head_dim), jnp.uint32),
            pltpu.VMEM((d_model // 2, d_ff), jnp.uint32),
            pltpu.VMEM((d_model // 2, d_ff), jnp.uint32),
            pltpu.VMEM((d_model // 2, d_ff), jnp.uint32),
            pltpu.VMEM((seq + 4 * seg, d_model), F32),
            pltpu.VMEM((seq + 4 * seg, d_model), BF16),
            pltpu.VMEM((2 * n_mem, d_model), F32),
            pltpu.VMEM((rows, n_heads * head_dim), BF16),
            pltpu.VMEM((4 * seg, d_ff), BF16),
            pltpu.VMEM((4 * seg, d_model // LANES * LANES), F32),
            pltpu.VMEM((d_model % LANES, 4 * seg), F32),
            pltpu.VMEM((rows // 2, rows // 2), F32),
            pltpu.VMEM((rows, rows), F32),
            pltpu.SemaphoreType.DMA((seq // LANES,)),
            pltpu.SemaphoreType.DMA((3, n_heads // 2)),
            pltpu.SemaphoreType.DMA((n_heads,)),
            pltpu.SemaphoreType.DMA((3,)),
            pltpu.SemaphoreType.DMA((seq // LANES,)),
        ],
        compiler_params=pltpu.CompilerParams(vmem_limit_bytes=100 * 1024 * 1024),
    )(
        A_x[0].T,
        A_mem0[0],
        A_Wq,
        A_Wk,
        A_Wv,
        jnp.transpose(A_Wo, (0, 2, 1)),
        B_w1,
        B_w3,
        B_w2.T,
    )
    return out_t.T[None]
```
